```python
import os as _os
_os.environ.setdefault("JAX_PLATFORMS", "cpu")
import jax
import jax.numpy as jnp

def _softmax(x, axis=-1):
    return jax.nn.softmax(x, axis=axis)
def _gelu(x):
    return jax.nn.gelu(x, approximate=True)
def _silu(x):
    return jax.nn.silu(x)
def _sigmoid(x):
    return jax.nn.sigmoid(x)
def _layernorm(x, axis=-1, eps=1e-5):
    m = jnp.mean(x, axis=axis, keepdims=True)
    v = jnp.var(x, axis=axis, keepdims=True)
    return (x - m) / jnp.sqrt(v + eps)
def _scatter_add(tgt, idx, src, axis=0):
    return tgt.at[idx].add(src)
def _segment_sum(src, seg, n):
    return jax.ops.segment_sum(src, seg, n)
class _Rng:
    def __init__(self, key):
        self._k = key
    def _next(self):
        self._k, sub = jax.random.split(self._k)
        return sub
    def normal(self, shape):
        return jax.random.normal(self._next(), shape, dtype=jnp.bfloat16)
    def randint(self, lo, hi, shape):
        return jax.random.randint(self._next(), shape, lo, hi, dtype=jnp.int32)
    def uniform(self, shape, lo=0.0, hi=1.0):
        return jax.random.uniform(self._next(), shape, jnp.bfloat16, lo, hi)
    def permutation(self, n):
        return jax.random.permutation(self._next(), n)


kernel_name = 'sequential_preLN__mha_block__swiglu_ffn__prompt'

def setup_inputs():
    _rng = _Rng(jax.random.key(int.from_bytes(__import__("os").urandom(4), "little")))
    _w = (lambda a: (lambda t: t.astype(jnp.bfloat16) if jnp.issubdtype(t.dtype, jnp.floating) else t)(jnp.asarray(a)))
    def _A_setup():
        B, S, D, H = 1, 2048, 640, 32
        return {
            "x": _w((lambda *s: _rng.normal(s) * 0.05)(B, S, D)),
            "wqkv": _w((lambda *s: _rng.normal(s) * 0.05)(D, 3 * D)),
            "wo": _w((lambda *s: _rng.normal(s) * 0.05)(D, D)),
        }
    _A_in = _A_setup()

    def _B_setup():
        B, S, D, F = 1, 2048, 640, 1728
        return {
            "x": _w((lambda *s: _rng.normal(s) * 0.05)(B, S, D)),
            "w_gate": _w((lambda *s: _rng.normal(s) * 0.05)(D, F)),
            "w_up": _w((lambda *s: _rng.normal(s) * 0.05)(D, F)),
            "w_down": _w((lambda *s: _rng.normal(s) * 0.05)(F, D)),
        }
    _B_in = _B_setup()

    return {
        "A_x": _A_in["x"],
        "A_wqkv": _A_in["wqkv"],
        "A_wo": _A_in["wo"],
        "B_x": _B_in["x"],
        "B_w_gate": _B_in["w_gate"],
        "B_w_up": _B_in["w_up"],
        "B_w_down": _B_in["w_down"],
    }

def reference(A_x, A_wqkv, A_wo, B_x, B_w_gate, B_w_up, B_w_down):
    def _A_ref(x, wqkv, wo):
        B, S, D = x.shape
        H = 32
        Dh = D // H
        qkv = (lambda x, *d: x.transpose(*d))((x @ wqkv).reshape(B, S, 3, H, Dh), 2, 0, 3, 1, 4)
        q, k, v = qkv[0], qkv[1], qkv[2]
        scores = jnp.einsum("bhqd,bhkd->bhqk", q, k) * (Dh ** -0.5)
        p = _softmax(scores, axis=-1)
        o = jnp.einsum("bhqk,bhkd->bhqd", p, v)
        return (lambda x, *d: x.transpose(*d))(o, 0, 2, 1, 3).reshape(B, S, D) @ wo

    def _B_ref(x, w_gate, w_up, w_down):
        g = _silu(x @ w_gate)
        u = x @ w_up
        return (g * u) @ w_down

    x = A_x
    h = x + _A_ref(_layernorm(x, axis=-1), A_wqkv, A_wo)
    h2 = h + _B_ref(_layernorm(h, axis=-1), B_w_gate, B_w_up, B_w_down)
    return h2
```

```python
import functools
import math

import jax
import jax.numpy as jnp
from jax import lax
import jax.experimental.pallas as pl
import jax.experimental.pallas.tpu as pltpu

_H = 32
_EPS = 1e-5
_LANES = 128
_TQ = 512
_RC = 512

_NT = (((1,), (1,)), ((), ()))


def _layernorm_f32(x):
    m = jnp.mean(x, axis=-1, keepdims=True)
    xc = x - m
    v = jnp.mean(xc * xc, axis=-1, keepdims=True)
    return xc * lax.rsqrt(v + _EPS)


def _kernel(x_ref, wqkv_ref, wo_ref, wg_ref, wu_ref, wd_ref, o_ref,
            wqk_scr, wvt_scr, q_scr, k_scr, vx_scr, ot_scr,
            *, S, D, F, DH, HPS, NSLAB):
    step = pl.program_id(0)
    qscale = (DH ** -0.5) * math.log2(math.e)

    @pl.when(step == 0)
    def _():
        w = wqkv_ref[...]
        for part in range(2):
            for s in range(NSLAB):
                a = s * HPS * DH
                n = min(HPS * DH, D - a)
                blk = w[:, part * D + a: part * D + a + n]
                blk = jnp.concatenate(
                    [blk, jnp.zeros((D, _LANES - n), w.dtype)], axis=1)
                c = (part * NSLAB + s) * _LANES
                wqk_scr[:, c:c + _LANES] = blk
        wvt_scr[...] = w[:, 2 * D:].astype(jnp.float32).T.astype(w.dtype)

        row32 = lax.broadcasted_iota(jnp.int32, (32, _RC), 0)

        def chunk(c, carry):
            r0 = pl.multiple_of(c * _RC, _RC)
            xn = _layernorm_f32(x_ref[pl.ds(r0, _RC), :].astype(jnp.float32))
            xn = xn.astype(jnp.bfloat16)
            qk = jnp.dot(xn, wqk_scr[...], preferred_element_type=jnp.float32)
            for s in range(NSLAB):
                q_scr[s, pl.ds(r0, _RC), :] = (
                    qk[:, s * _LANES:(s + 1) * _LANES] * qscale
                ).astype(jnp.bfloat16)
                k_scr[s, pl.ds(r0, _RC), :] = (
                    qk[:, (NSLAB + s) * _LANES:(NSLAB + s + 1) * _LANES]
                ).astype(jnp.bfloat16)
            vt = lax.dot_general(wvt_scr[...], xn, _NT,
                                 preferred_element_type=jnp.float32)
            for h in range(_H):
                w0 = 16 * ((DH * h) // 16)
                ones_row = 31 if (DH * h) % 16 == 0 else 0
                win = jnp.where(row32 == ones_row, 1.0, vt[w0:w0 + 32, :])
                vx_scr[h, :, pl.ds(r0, _RC)] = win.astype(jnp.bfloat16)
            return carry

        lax.fori_loop(0, S // _RC, chunk, 0)

    q0 = pl.multiple_of(step * _TQ, _TQ)
    lane = lax.broadcasted_iota(jnp.int32, (_TQ, _LANES), 1)
    row32q = lax.broadcasted_iota(jnp.int32, (32, _TQ), 0)

    def head(h, carry):
        slab = h // HPS
        lo = (h % HPS) * DH
        q = q_scr[slab, pl.ds(q0, _TQ), :]
        qm = jnp.where((lane >= lo) & (lane < lo + DH), q, jnp.zeros_like(q))
        st = lax.dot_general(k_scr[slab], qm, _NT,
                             preferred_element_type=jnp.float32)
        m = jnp.max(st, axis=0, keepdims=True)
        p = jnp.exp2(st - m).astype(jnp.bfloat16)
        o = jnp.dot(vx_scr[h], p, preferred_element_type=jnp.float32)
        off = (DH * h) % 16
        w0 = pl.multiple_of(DH * h - off, 16)
        l = jnp.where(off == 0, o[31:32, :], o[0:1, :])
        on = o * (1.0 / l)
        valid = (row32q >= off) & (row32q < off + DH)
        pltpu.store(ot_scr.at[pl.ds(w0, 32), :], on, mask=valid)
        return carry

    lax.fori_loop(0, _H, head, 0)

    o_nat = ot_scr[...].T.astype(jnp.bfloat16)
    attn = jnp.dot(o_nat, wo_ref[...], preferred_element_type=jnp.float32)
    hres = x_ref[pl.ds(q0, _TQ), :].astype(jnp.float32) + attn
    hn = _layernorm_f32(hres).astype(jnp.bfloat16)
    g = jnp.dot(hn, wg_ref[...], preferred_element_type=jnp.float32)
    u = jnp.dot(hn, wu_ref[...], preferred_element_type=jnp.float32)
    act = (g * jax.nn.sigmoid(g) * u).astype(jnp.bfloat16)
    dn = jnp.dot(act, wd_ref[...], preferred_element_type=jnp.float32)
    o_ref[...] = (hres + dn).astype(o_ref.dtype)


@jax.jit
def pallas_sequential_preLN__mha_block__swiglu_ffn__prompt_kernel(
    A_x: jax.Array,
    A_wqkv: jax.Array,
    A_wo: jax.Array,
    B_x: jax.Array,
    B_w_gate: jax.Array,
    B_w_up: jax.Array,
    B_w_down: jax.Array,
):
    del B_x
    B, S, D = A_x.shape
    assert B == 1
    F = B_w_gate.shape[1]
    DH = D // _H
    HPS = _LANES // DH
    NSLAB = -(-_H // HPS)
    x = A_x.reshape(S, D)

    kern = functools.partial(_kernel, S=S, D=D, F=F, DH=DH, HPS=HPS,
                             NSLAB=NSLAB)
    full = lambda shape: pl.BlockSpec(shape, lambda i: (0,) * len(shape))
    out = pl.pallas_call(
        kern,
        grid=(S // _TQ,),
        in_specs=[
            full((S, D)),
            full((D, 3 * D)),
            full((D, D)),
            full((D, F)),
            full((D, F)),
            full((F, D)),
        ],
        out_specs=pl.BlockSpec((_TQ, D), lambda i: (i, 0)),
        out_shape=jax.ShapeDtypeStruct((S, D), A_x.dtype),
        scratch_shapes=[
            pltpu.VMEM((D, 2 * NSLAB * _LANES), jnp.bfloat16),
            pltpu.VMEM((D, D), jnp.bfloat16),
            pltpu.VMEM((NSLAB, S, _LANES), jnp.bfloat16),
            pltpu.VMEM((NSLAB, S, _LANES), jnp.bfloat16),
            pltpu.VMEM((_H, 32, S), jnp.bfloat16),
            pltpu.VMEM((D, _TQ), jnp.float32),
        ],
        compiler_params=pltpu.CompilerParams(
            dimension_semantics=("arbitrary",),
            vmem_limit_bytes=100 * 1024 * 1024,
        ),
    )(x, A_wqkv, A_wo, B_w_gate, B_w_up, B_w_down)
    return out.reshape(B, S, D)
```

```python
import functools
import math

import jax
import jax.numpy as jnp
from jax import lax
import jax.experimental.pallas as pl
import jax.experimental.pallas.tpu as pltpu

_H = 32
_EPS = 1e-5
_LANES = 128
_TQ = 512
_KC = 128
_UN = 4
_VR = 24
_FS = 2

_NN = (((1,), (0,)), ((), ()))
_NT = (((1,), (1,)), ((), ()))


def _layernorm_f32(x):
    m = jnp.mean(x, axis=-1, keepdims=True)
    xc = x - m
    v = jnp.mean(xc * xc, axis=-1, keepdims=True)
    return xc * lax.rsqrt(v + _EPS)


def _kernel(x_hbm, wqkv_hbm, wo_hbm, wgt_hbm, wut_hbm, wd_hbm, o_ref,
            x_v, w3_v, wo_v, wgu_v, wd_v,
            xn_scr, wqvt_scr, qm_scr, k_scr, vx_scr, ot_scr, sa_scr, sb_scr,
            m_scr, sems, *, S, D, F, DH, HPS, NSLAB):
    step = pl.program_id(0)
    qscale = (DH ** -0.5) * math.log2(math.e)
    TQ, KC = _TQ, _KC
    NC = S // KC
    NQ = S // TQ
    FM = (F // _LANES) * _LANES
    FT = F - FM
    bf16 = jnp.bfloat16
    f32 = jnp.float32

    def x_copy(c):
        return pltpu.make_async_copy(
            x_hbm.at[pl.ds(c * TQ, TQ), :], x_v.at[pl.ds(c * TQ, TQ), :],
            sems.at[c])

    def w3_copy(j):
        return pltpu.make_async_copy(
            wqkv_hbm.at[:, pl.ds(j * D, D)], w3_v.at[j], sems.at[NQ + j])

    def late_copies():
        b = NQ + 3
        return [
            pltpu.make_async_copy(wo_hbm, wo_v, sems.at[b]),
            pltpu.make_async_copy(wgt_hbm.at[pl.ds(0, FM), :],
                                  wgu_v.at[pl.ds(0, FM), :], sems.at[b + 1]),
            pltpu.make_async_copy(wut_hbm.at[pl.ds(0, FM), :],
                                  wgu_v.at[pl.ds(FM, FM), :], sems.at[b + 2]),
            pltpu.make_async_copy(wgt_hbm.at[pl.ds(FM, FT), :],
                                  wgu_v.at[pl.ds(2 * FM, FT), :],
                                  sems.at[b + 3]),
            pltpu.make_async_copy(wut_hbm.at[pl.ds(FM, FT), :],
                                  wgu_v.at[pl.ds(2 * FM + FT, FT), :],
                                  sems.at[b + 4]),
            pltpu.make_async_copy(wd_hbm, wd_v, sems.at[b + 5]),
        ]

    rowv = lax.broadcasted_iota(jnp.int32, (_VR, TQ), 0)

    def scores_chunk(h, qb, c, s_dst, mrun):
        st = jnp.dot(k_scr[h // HPS, c * KC:(c + 1) * KC, :], qm_scr[qb, h],
                     preferred_element_type=f32)
        s_dst[c * KC:(c + 1) * KC, :] = st
        cm = jnp.max(st.reshape(KC // 8, 8, TQ), axis=0)
        return cm if mrun is None else jnp.maximum(mrun, cm)

    def pv_chunk(h, c, s_src, m, acc):
        z = pl.multiple_of(lax.shift_right_logical(h, 10) * KC, KC)
        p = jnp.exp2(s_src[pl.ds(z + c * KC, KC), :] - m).astype(bf16)
        o = lax.dot_general(vx_scr[h, :, c * KC:(c + 1) * KC], p, _NN,
                            preferred_element_type=f32)
        return o if acc is None else acc + o

    def finish(h, o):
        off = (DH * h) % 8
        w0 = pl.multiple_of(DH * h - off, 8)
        l = jnp.where(off == 0, o[_VR - 1:_VR, :], o[0:1, :])
        on = o * (1.0 / l)
        valid = (rowv >= off) & (rowv < off + DH)
        pltpu.store(ot_scr.at[pl.ds(w0, _VR), :], on, mask=valid)

    def unit(h_cur, h_next, qb_next, s_cur, s_next, m_cur):
        mrun = None
        acc = None
        for c in range(NC):
            mrun = scores_chunk(h_next, qb_next, c, s_next, mrun)
            if h_cur is not None:
                acc = pv_chunk(h_cur, c, s_cur, m_cur, acc)
        if h_cur is not None:
            finish(h_cur, acc)
        return jnp.max(mrun, axis=0, keepdims=True)

    @pl.when(step == 0)
    def _():
        x_copy(0).start()
        w3_copy(1).start()
        for c in range(1, NQ):
            x_copy(c).start()
        w3_copy(0).start()
        w3_copy(2).start()

        def zero_fill(qb, carry):
            for h in range(_H):
                g0 = 16 * (((h % HPS) * DH) // 16)
                if g0 > 0:
                    qm_scr[qb, h, 0:g0, :] = jnp.zeros((g0, TQ), bf16)
                if g0 + 32 < _LANES:
                    qm_scr[qb, h, g0 + 32:, :] = jnp.zeros(
                        (_LANES - g0 - 32, TQ), bf16)
            return carry
        lax.fori_loop(0, NQ, zero_fill, 0)

        def ln1(c):
            x_copy(c).wait()
            xn_scr[c * TQ:(c + 1) * TQ, :] = _layernorm_f32(
                x_v[c * TQ:(c + 1) * TQ, :].astype(f32)).astype(bf16)

        def wt(j, dst):
            w3_copy(j).wait()
            wqvt_scr[dst * D:(dst + 1) * D, :] = (
                w3_v[j].astype(f32).T.astype(bf16))

        ln1(0)
        w3_copy(1).wait()
        for c in range(NQ):
            if c + 1 < NQ:
                ln1(c + 1)
            if c == 1:
                wt(0, 0)
            if c == 2:
                wt(2, 1)
                for cp in late_copies():
                    cp.start()
            k = jnp.dot(xn_scr[c * TQ:(c + 1) * TQ, :], w3_v[1],
                        preferred_element_type=f32).astype(bf16)
            for s in range(NSLAB):
                a = s * HPS * DH
                if a + _LANES <= D:
                    blk = k[:, a:a + _LANES]
                else:
                    blk = jnp.concatenate(
                        [k[:, a:], jnp.zeros((TQ, a + _LANES - D), bf16)],
                        axis=1)
                k_scr[s, c * TQ:(c + 1) * TQ, :] = blk

        row32 = lax.broadcasted_iota(jnp.int32, (32, TQ), 0)

        def chunk(c, carry):
            r0 = pl.multiple_of(c * TQ, TQ)
            qvt = lax.dot_general(wqvt_scr[...], xn_scr[pl.ds(r0, TQ), :], _NT,
                                  preferred_element_type=f32)
            vt = qvt[D:, :].astype(bf16).astype(f32)
            for h in range(_H):
                lo = (h % HPS) * DH
                g0 = 16 * (lo // 16)
                src = h * DH - (lo - g0)
                win = qvt[src:src + 32, :] * qscale
                keep = (row32 >= lo - g0) & (row32 < lo - g0 + DH)
                qm_scr[c, h, g0:g0 + 32, :] = (
                    jnp.where(keep, win, 0.0).astype(bf16))
                w0 = 8 * ((DH * h) // 8)
                ones_row = _VR - 1 if (DH * h) % 8 == 0 else 0
                win = jnp.where(rowv == ones_row, 1.0, vt[w0:w0 + _VR, :])
                vx_scr[h, :, pl.ds(r0, TQ)] = win
            return carry

        lax.fori_loop(0, NQ, chunk, 0)
        m_scr[...] = unit(None, 0, 0, None, sa_scr, None)

    def body(i, m):
        h = i * _UN
        for j in range(_UN):
            cur, nxt = (sa_scr, sb_scr) if j % 2 == 0 else (sb_scr, sa_scr)
            hn = h + j + 1
            if j == _UN - 1:
                qb = jnp.minimum(step + hn // _H, NQ - 1)
                hn = hn % _H
            else:
                qb = step
            m = unit(h + j, hn, qb, cur, nxt, m)
        return m

    m_scr[...] = lax.fori_loop(0, _H // _UN, body, m_scr[...])

    @pl.when(step == 0)
    def _():
        for cp in late_copies():
            cp.wait()

    R = TQ // _FS
    hres = []
    for r in range(_FS):
        o_nat = ot_scr[:, r * R:(r + 1) * R].T.astype(bf16)
        attn = jnp.dot(o_nat, wo_v[...], preferred_element_type=f32)
        q0 = pl.multiple_of(step * TQ + r * R, R)
        hres.append(x_v[pl.ds(q0, R), :].astype(f32) + attn)
    for r in range(_FS):
        hn = _layernorm_f32(hres[r]).astype(bf16)
        gu = lax.dot_general(hn, wgu_v[...], _NT, preferred_element_type=f32)
        g = jnp.concatenate([gu[:, 0:FM], gu[:, 2 * FM:2 * FM + FT]], axis=1)
        u = jnp.concatenate([gu[:, FM:2 * FM], gu[:, 2 * FM + FT:]], axis=1)
        act = (g * jax.nn.sigmoid(g) * u).astype(bf16)
        dn = jnp.dot(act, wd_v[...], preferred_element_type=f32)
        o_ref[r * R:(r + 1) * R, :] = (hres[r] + dn).astype(o_ref.dtype)


@jax.jit
def pallas_sequential_preLN__mha_block__swiglu_ffn__prompt_kernel(
    A_x: jax.Array,
    A_wqkv: jax.Array,
    A_wo: jax.Array,
    B_x: jax.Array,
    B_w_gate: jax.Array,
    B_w_up: jax.Array,
    B_w_down: jax.Array,
):
    del B_x
    B, S, D = A_x.shape
    assert B == 1
    F = B_w_gate.shape[1]
    DH = D // _H
    HPS = _LANES // DH
    NSLAB = -(-_H // HPS)
    NQ = S // _TQ
    x = A_x.reshape(S, D)
    bf16 = jnp.bfloat16

    kern = functools.partial(_kernel, S=S, D=D, F=F, DH=DH, HPS=HPS,
                             NSLAB=NSLAB)
    out = pl.pallas_call(
        kern,
        grid=(NQ,),
        in_specs=[pl.BlockSpec(memory_space=pl.ANY)] * 6,
        out_specs=pl.BlockSpec((_TQ, D), lambda i: (i, 0)),
        out_shape=jax.ShapeDtypeStruct((S, D), A_x.dtype),
        scratch_shapes=[
            pltpu.VMEM((S, D), bf16),
            pltpu.VMEM((3, D, D), bf16),
            pltpu.VMEM((D, D), bf16),
            pltpu.VMEM((2 * F, D), bf16),
            pltpu.VMEM((F, D), bf16),
            pltpu.VMEM((S, D), bf16),
            pltpu.VMEM((2 * D, D), bf16),
            pltpu.VMEM((NQ, _H, _LANES, _TQ), bf16),
            pltpu.VMEM((NSLAB, S, _LANES), bf16),
            pltpu.VMEM((_H, _VR, S), jnp.float32),
            pltpu.VMEM((D, _TQ), jnp.float32),
            pltpu.VMEM((S, _TQ), jnp.float32),
            pltpu.VMEM((S, _TQ), jnp.float32),
            pltpu.VMEM((1, _TQ), jnp.float32),
            pltpu.SemaphoreType.DMA((NQ + 9,)),
        ],
        compiler_params=pltpu.CompilerParams(
            dimension_semantics=("arbitrary",),
            vmem_limit_bytes=100 * 1024 * 1024,
        ),
    )(x, A_wqkv, A_wo, B_w_gate.T, B_w_up.T, B_w_down)
    return out.reshape(B, S, D)
```

```python
import functools
import math

import jax
import jax.numpy as jnp
from jax import lax
import jax.experimental.pallas as pl
import jax.experimental.pallas.tpu as pltpu

_H = 32
_EPS = 1e-5
_LANES = 128
_TQ = 512
_KC = 128
_VR = 24
_LAG = 1
_NV = 128
_VG = 8
_FS = 2
_PF32 = True
_BA = 1
_LP = 2
_VE = 0
_TR = 0
_TV = 16

_NN = (((1,), (0,)), ((), ()))
_NT = (((1,), (1,)), ((), ()))


def _layernorm_f32(x):
    m = jnp.mean(x, axis=-1, keepdims=True)
    xc = x - m
    v = jnp.mean(xc * xc, axis=-1, keepdims=True)
    return xc * lax.rsqrt(v + _EPS)


def _kernel(x_hbm, wqkv_hbm, wo_hbm, wgt_hbm, wut_hbm, wd_hbm, o_ref,
            x_v, w3_v, wo_v, wgu_v, wd_v,
            xn_scr, wqvt_scr, qm_scr, k_scr, vx_scr, ot_scr, s0_scr, s1_scr,
            s2_scr, s3_scr,
            kv_scr, qf_scr, kb_scr, sems, *, S, D, F, DH, HPS, NSLAB):
    step = pl.program_id(0)
    s_scr = (s0_scr, s1_scr, s2_scr, s3_scr)
    qscale = (DH ** -0.5) * math.log2(math.e)
    TQ, KC = _TQ, _KC
    NC = S // KC
    NQ = S // TQ
    NJ = TQ // _LANES
    FM = (F // _LANES) * _LANES
    FT = F - FM
    bf16 = jnp.bfloat16
    f32 = jnp.float32
    u32 = jnp.uint32
    NM = NC
    NG = _NV // _VG
    n16 = _NV // 16
    vchunks = [c for c in range(NC)
               if ((c + 1) * n16) // NC > (c * n16) // NC]
    assert len(vchunks) == n16
    vrow = [vc * KC + KC - 16 + o for vc in vchunks for o in (0, 8)]

    def x_copy(c):
        return pltpu.make_async_copy(
            x_hbm.at[pl.ds(c * TQ, TQ), :], x_v.at[pl.ds(c * TQ, TQ), :],
            sems.at[c])

    def w3_copy(j):
        return pltpu.make_async_copy(
            wqkv_hbm.at[:, pl.ds(j * D, D)], w3_v.at[j], sems.at[NQ + j])

    def late_copies():
        b = NQ + 3
        return [
            pltpu.make_async_copy(wo_hbm, wo_v, sems.at[b]),
            pltpu.make_async_copy(wgt_hbm.at[pl.ds(0, FM), :],
                                  wgu_v.at[pl.ds(0, FM), :], sems.at[b + 1]),
            pltpu.make_async_copy(wut_hbm.at[pl.ds(0, FM), :],
                                  wgu_v.at[pl.ds(FM, FM), :], sems.at[b + 2]),
            pltpu.make_async_copy(wgt_hbm.at[pl.ds(FM, FT), :],
                                  wgu_v.at[pl.ds(2 * FM, FT), :],
                                  sems.at[b + 3]),
            pltpu.make_async_copy(wut_hbm.at[pl.ds(FM, FT), :],
                                  wgu_v.at[pl.ds(2 * FM + FT, FT), :],
                                  sems.at[b + 4]),
            pltpu.make_async_copy(wd_hbm, wd_v, sems.at[b + 5]),
        ]

    rowv = lax.broadcasted_iota(jnp.int32, (_VR, TQ), 0)
    row8 = lax.broadcasted_iota(jnp.int32, (8, TQ), 0)
    row8l = lax.broadcasted_iota(jnp.int32, (8, _LANES), 0)

    def scores_chunk(h, qb, c, s_dst, mrun):
        n = KC - 16 if c in vchunks else KC
        kc = pltpu.bitcast(
            k_scr[h // HPS, c * KC // 2:(c * KC + n) // 2, :], bf16)
        st = jnp.dot(kc, pltpu.bitcast(qm_scr[qb, h], bf16),
                     preferred_element_type=f32)
        s_dst[c * KC:c * KC + n, :] = st
        cm = jnp.max(st.reshape(n // 8, 8, TQ), axis=0)
        return ((cm if mrun is None else jnp.maximum(mrun, cm)),
                st[_TR:_TR + 8, :], st[_TV:_TV + 8, :])

    def scores_vpu(h, qb, g, s_dst, mrun, start):
        z = lax.shift_right_logical(h, 10)
        acc = [None] * NJ
        for d in range(DH):
            kb = kb_scr[z + (g * DH + d)]
            for j in range(NJ):
                t = kb * qf_scr[qb, h, d:d + 1, j * _LANES:(j + 1) * _LANES]
                if acc[j] is None and start is not None:
                    zs = lax.shift_right_logical(h + 300, 10)
                    t = jnp.where(row8l < zs,
                                  start[:, j * _LANES:(j + 1) * _LANES], t)
                acc[j] = t if acc[j] is None else acc[j] + t
        st = jnp.concatenate(acc, axis=1)
        r0 = vrow[g]
        s_dst[r0:r0 + _VG, :] = st
        cm = jnp.max(st.reshape(_VG // 8, 8, TQ), axis=0)
        return (cm if mrun is None else jnp.maximum(mrun, cm)), st

    def build_kb(h, g):
        kh = kv_scr[h, g * _VG:(g + 1) * _VG, :]
        for d in range(DH):
            kb_scr[g * DH + d] = jnp.broadcast_to(
                kh[:, d:d + 1], (_VG, _LANES)).astype(f32)

    def pv_chunk(h, c, s_src, m, acc, tie):
        z = pl.multiple_of(lax.shift_right_logical(h, 10) * KC, KC)
        if tie is not None:
            for i, t in enumerate(tie):
                zi = lax.shift_right_logical(h + (200 + i), 10)
                m = jnp.where(row8 < zi, t, m)
        sv = s_src[pl.ds(z + c * KC, KC), :].reshape(KC // 8, 8, TQ)
        p = jnp.exp2(sv - m[None]).reshape(KC, TQ)
        if not _PF32:
            p = p.astype(bf16)
        o = lax.dot_general(vx_scr[h, :, c * KC:(c + 1) * KC], p, _NN,
                            preferred_element_type=f32)
        return o if acc is None else o + acc

    def finish(h, qb, o):
        off = (DH * h) % 8
        w0 = pl.multiple_of(DH * h - off, 8)
        l = jnp.where(off == 0, o[_VR - 1:_VR, :], o[0:1, :])
        on = o * (1.0 / l)
        valid = (rowv >= off) & (rowv < off + DH)
        pltpu.store(ot_scr.at[qb, pl.ds(w0, _VR), :], on, mask=valid)

    def a_unit_items(nxt, s_next, build, gstate):
        state = {"mrun": None, "mv": None}
        slots = []
        gdone = 0
        bdone = 0
        span = NM - _VE
        for c in range(NM):
            gs, bs = [], []
            while gdone < NG and gdone * span < (c + 1) * NG:
                while build and bdone < min(NG, gdone + 1 + _BA):
                    bs.append(bdone)
                    bdone += 1
                gs.append(gdone)
                gdone += 1

            def run(c=c, gs=tuple(gs), bs=tuple(bs)):
                state["mrun"], tie, mid = scores_chunk(
                    nxt[0], nxt[1], c, s_next, state["mrun"])
                tie = (tie,)
                start = gstate.get("mid")
                gstate["mid"] = mid
                for g in bs:
                    build_kb(nxt[0], g)
                for g in gs:
                    state["mv"], vt = scores_vpu(
                        nxt[0], nxt[1], g, s_next, state["mv"], start)
                    tie = tie + (vt,)
                return tie
            slots.append(run)

        def final():
            mm = state["mrun"]
            if state["mv"] is not None:
                mm = jnp.maximum(mm, state["mv"])
            return jnp.broadcast_to(
                jnp.max(mm, axis=0, keepdims=True), (8, TQ))
        return slots, final

    @pl.when(step == 0)
    def _():
        x_copy(0).start()
        w3_copy(1).start()
        for c in range(1, NQ):
            x_copy(c).start()
        w3_copy(0).start()
        w3_copy(2).start()

        def zero_fill(qb, carry):
            for h in range(_H):
                g0 = 16 * (((h % HPS) * DH) // 16)
                if g0 > 0:
                    qm_scr[qb, h, 0:g0 // 2, :] = jnp.zeros((g0 // 2, TQ), u32)
                if g0 + 32 < _LANES:
                    qm_scr[qb, h, g0 // 2 + 16:, :] = jnp.zeros(
                        ((_LANES - g0 - 32) // 2, TQ), u32)
            return carry
        lax.fori_loop(0, NQ, zero_fill, 0)

        def ln1(c):
            xn_scr[c * TQ:(c + 1) * TQ, :] = _layernorm_f32(
                x_v[c * TQ:(c + 1) * TQ, :].astype(f32)).astype(bf16)

        def wt(j, dst):
            wqvt_scr[dst * D:(dst + 1) * D, :] = (
                w3_v[j].astype(f32).T.astype(bf16))

        def kproj(c):
            k = jnp.dot(xn_scr[c * TQ:(c + 1) * TQ, :], w3_v[1],
                        preferred_element_type=f32).astype(bf16)
            for s in range(NSLAB):
                a = s * HPS * DH
                if a + _LANES <= D:
                    blk = k[:, a:a + _LANES]
                else:
                    blk = jnp.concatenate(
                        [k[:, a:], jnp.zeros((TQ, a + _LANES - D), bf16)],
                        axis=1)
                k_scr[s, c * TQ // 2:(c + 1) * TQ // 2, :] = (
                    pltpu.bitcast(blk, u32))
            mine = [i for i, vc in enumerate(vchunks)
                    if vc * KC // TQ == c]
            if mine:
                kt = jnp.concatenate(
                    [k[vrow[2 * i] - c * TQ:vrow[2 * i] - c * TQ + 16, :]
                     for i in mine], axis=0).astype(f32)
                kt = jnp.concatenate(
                    [kt, jnp.zeros((kt.shape[0], _LANES), f32)], axis=1)
                for h in range(_H):
                    kv_scr[h, 16 * mine[0]:16 * (mine[-1] + 1), :] = (
                        kt[:, h * DH:h * DH + _LANES])

        x_copy(0).wait()
        ln1(0)
        w3_copy(1).wait()
        x_copy(1).wait()
        ln1(1)
        kproj(0)
        x_copy(2).wait()
        x_copy(3).wait()
        ln1(2)
        ln1(3)
        kproj(1)
        w3_copy(0).wait()
        w3_copy(2).wait()
        for cp in late_copies():
            cp.start()
        wt(0, 0)
        wt(2, 1)
        kproj(2)
        kproj(3)

        row32 = lax.broadcasted_iota(jnp.int32, (32, TQ), 0)

        def chunk(c, carry):
            r0 = pl.multiple_of(c * TQ, TQ)
            qvt = lax.dot_general(wqvt_scr[...], xn_scr[pl.ds(r0, TQ), :], _NT,
                                  preferred_element_type=f32)
            vt = qvt[D:, :]
            qs = (qvt[0:D + 32, :] * qscale).astype(bf16).astype(f32)
            for h in range(_H):
                lo = (h % HPS) * DH
                g0 = 16 * (lo // 16)
                src = h * DH - (lo - g0)
                keep = (row32 >= lo - g0) & (row32 < lo - g0 + DH)
                qm_scr[c, h, g0 // 2:g0 // 2 + 16, :] = pltpu.bitcast(
                    jnp.where(keep, qs[src:src + 32, :], 0.0).astype(bf16),
                    u32)
                qf_scr[c, h] = qs[h * DH:h * DH + _VR, :]
                w0 = 8 * ((DH * h) // 8)
                ones_row = _VR - 1 if (DH * h) % 8 == 0 else 0
                win = jnp.where(rowv == ones_row, 1.0, vt[w0:w0 + _VR, :])
                vx_scr[h, :, pl.ds(r0, TQ)] = win
            return carry

        lax.fori_loop(0, NQ, chunk, 0)
        slots, final = a_unit_items((step, 0), s_scr[0], True, {})
        for run in slots:
            run()
        m0 = final()
        s_scr[NQ - 1][(NC - _LP) * KC:, :] = jnp.zeros((_LP * KC, TQ), f32)

        def body(h, carry):
            m_prev, acc_prev, m_cur = carry
            hp = jnp.maximum(h - 1, 0)
            hn = jnp.minimum(h + 1, _H - 1)
            ms = {-1: m_prev, 0: m_cur}
            accs = {-1: acc_prev}
            pv_at = {}
            for p in range(-_LP, NQ * NC - _LP):
                pv_at.setdefault(((p + _LP) * NM) // NC, []).append(p)
            tie = None
            gstate = {}
            for j in range(NQ):
                nu = (h, j + 1) if j + 1 < NQ else (hn, 0)
                slots, final = a_unit_items(nu, s_scr[(j + 1) % NQ],
                                            j + 1 == NQ, gstate)
                for c in range(NM):
                    new_tie = slots[c]()
                    for p in pv_at.get(j * NM + c, []):
                        u, pc = p // NC, p % NC
                        hu = hp if u < 0 else h
                        accs[u] = pv_chunk(hu, pc, s_scr[u % NQ], ms[u],
                                           accs.get(u), tie)
                        if pc == NC - 1:
                            finish(hu, u % NQ, accs[u])
                    tie = new_tie
                ms[j + 1] = final()
            return ms[NQ - 1], accs[NQ - 1], ms[NQ]

        m_prev, acc_prev, _ = lax.fori_loop(
            0, _H, body,
            (jnp.zeros((8, TQ), f32), jnp.zeros((_VR, TQ), f32), m0))
        hl = _H - 1 + step
        for pc in range(NC - _LP, NC):
            acc_prev = pv_chunk(hl, pc, s_scr[NQ - 1], m_prev, acc_prev, None)
        finish(hl, NQ - 1, acc_prev)
        for cp in late_copies():
            cp.wait()

    R = TQ // _FS
    hres = []
    for r in range(_FS):
        o_nat = ot_scr[step, :, r * R:(r + 1) * R].T.astype(bf16)
        attn = jnp.dot(o_nat, wo_v[...], preferred_element_type=f32)
        q0 = pl.multiple_of(step * TQ + r * R, R)
        hres.append(x_v[pl.ds(q0, R), :].astype(f32) + attn)
    for r in range(_FS):
        hn = _layernorm_f32(hres[r]).astype(bf16)
        gu = lax.dot_general(hn, wgu_v[...], _NT, preferred_element_type=f32)
        g = jnp.concatenate([gu[:, 0:FM], gu[:, 2 * FM:2 * FM + FT]], axis=1)
        u = jnp.concatenate([gu[:, FM:2 * FM], gu[:, 2 * FM + FT:]], axis=1)
        act = (g * jax.nn.sigmoid(g) * u).astype(bf16)
        dn = jnp.dot(act, wd_v[...], preferred_element_type=f32)
        o_ref[r * R:(r + 1) * R, :] = (hres[r] + dn).astype(o_ref.dtype)


@jax.jit
def pallas_sequential_preLN__mha_block__swiglu_ffn__prompt_kernel(
    A_x: jax.Array,
    A_wqkv: jax.Array,
    A_wo: jax.Array,
    B_x: jax.Array,
    B_w_gate: jax.Array,
    B_w_up: jax.Array,
    B_w_down: jax.Array,
):
    del B_x
    B, S, D = A_x.shape
    assert B == 1
    F = B_w_gate.shape[1]
    DH = D // _H
    HPS = _LANES // DH
    NSLAB = -(-_H // HPS)
    NQ = S // _TQ
    x = A_x.reshape(S, D)
    bf16 = jnp.bfloat16
    f32 = jnp.float32

    kern = functools.partial(_kernel, S=S, D=D, F=F, DH=DH, HPS=HPS,
                             NSLAB=NSLAB)
    out = pl.pallas_call(
        kern,
        grid=(NQ,),
        in_specs=[pl.BlockSpec(memory_space=pl.ANY)] * 6,
        out_specs=pl.BlockSpec((_TQ, D), lambda i: (i, 0)),
        out_shape=jax.ShapeDtypeStruct((S, D), A_x.dtype),
        scratch_shapes=[
            pltpu.VMEM((S, D), bf16),
            pltpu.VMEM((3, D, D), bf16),
            pltpu.VMEM((D, D), bf16),
            pltpu.VMEM((2 * F, D), bf16),
            pltpu.VMEM((F, D), bf16),
            pltpu.VMEM((S, D), bf16),
            pltpu.VMEM((2 * D, D), bf16),
            pltpu.VMEM((NQ, _H, _LANES // 2, _TQ), jnp.uint32),
            pltpu.VMEM((NSLAB, S // 2, _LANES), jnp.uint32),
            pltpu.VMEM((_H, _VR, S), f32),
            pltpu.VMEM((NQ, D, _TQ), f32),
            pltpu.VMEM((S, _TQ), f32),
            pltpu.VMEM((S, _TQ), f32),
            pltpu.VMEM((S, _TQ), f32),
            pltpu.VMEM((S, _TQ), f32),
            pltpu.VMEM((_H, max(_NV, 8), _LANES), f32),
            pltpu.VMEM((NQ, _H, _VR, _TQ), f32),
            pltpu.VMEM((max(_NV // _VG, 1) * DH, _VG, _LANES), f32),
            pltpu.SemaphoreType.DMA((NQ + 9,)),
        ],
        compiler_params=pltpu.CompilerParams(
            dimension_semantics=("arbitrary",),
            vmem_limit_bytes=110 * 1024 * 1024,
        ),
    )(x, A_wqkv, A_wo, B_w_gate.T, B_w_up.T, B_w_down)
    return out.reshape(B, S, D)
```

```python
import functools
import math

import jax
import jax.numpy as jnp
from jax import lax
import jax.experimental.pallas as pl
import jax.experimental.pallas.tpu as pltpu

_H = 32
_EPS = 1e-5
_LANES = 128
_TQ = 512
_KC = 128
_VR = 24
_NV = 128
_FS = 2
_HU = 2
_LP = 2
_TE = (8, 56)
_TV = (48, 72)
_KM = 128
_DM = 1
_LNR = 64

_NN = (((1,), (0,)), ((), ()))
_NT = (((1,), (1,)), ((), ()))


def _layernorm_f32(x):
    m = jnp.mean(x, axis=-1, keepdims=True)
    xc = x - m
    v = jnp.mean(xc * xc, axis=-1, keepdims=True)
    return xc * lax.rsqrt(v + _EPS)


def _kernel(x_hbm, wqkv_hbm, wo_hbm, wgt_hbm, wut_hbm, wd_hbm, o_ref,
            x_v, wk_v, wqv_v, wo_v, wgu_v, wd_v,
            xn_scr, qm_scr, k_scr, vx_scr, ot_scr,
            s0_scr, s1_scr, s2_scr, s3_scr,
            kv_scr, qf_scr, kb0_scr, kb1_scr, kh0_scr, kh1_scr, sems,
            *, S, D, F, DH, HPS, NSLAB):
    step = pl.program_id(0)
    s_scr = (s0_scr, s1_scr, s2_scr, s3_scr)
    kb_scr = (kb0_scr, kb1_scr)
    kh_scr = (kh0_scr, kh1_scr)
    qscale = (DH ** -0.5) * math.log2(math.e)
    TQ, KC = _TQ, _KC
    NC = S // KC
    NQ = S // TQ
    NJ = TQ // _LANES
    FM = (F // _LANES) * _LANES
    FT = F - FM
    bf16 = jnp.bfloat16
    f32 = jnp.float32
    u32 = jnp.uint32
    NG = _NV // 8
    n16 = _NV // 16
    vchunks = [c for c in range(NC)
               if ((c + 1) * n16) // NC > (c * n16) // NC]
    vrow = [vc * KC + KC - 16 + o for vc in vchunks for o in (0, 8)]
    CPB = TQ // KC
    vloc = [vc for vc in vchunks if vc < CPB]
    assert vchunks == [b * CPB + v for b in range(NQ) for v in vloc]

    def opaque_zero(h, salt):
        return lax.shift_right_logical(h + salt, 10)

    def x_copy(c):
        return pltpu.make_async_copy(
            x_hbm.at[pl.ds(c * TQ, TQ), :], x_v.at[pl.ds(c * TQ, TQ), :],
            sems.at[c])

    def w_copies():
        return [
            pltpu.make_async_copy(wqkv_hbm.at[:, pl.ds(D, D)], wk_v,
                                  sems.at[NQ]),
            pltpu.make_async_copy(wqkv_hbm.at[:, pl.ds(0, D)],
                                  wqv_v.at[:, pl.ds(0, D)], sems.at[NQ + 1]),
            pltpu.make_async_copy(wqkv_hbm.at[:, pl.ds(2 * D, D)],
                                  wqv_v.at[:, pl.ds(D, D)], sems.at[NQ + 2]),
        ]

    def late_copies():
        b = NQ + 3
        return [
            pltpu.make_async_copy(wo_hbm, wo_v, sems.at[b]),
            pltpu.make_async_copy(wgt_hbm.at[pl.ds(0, FM), :],
                                  wgu_v.at[pl.ds(0, FM), :], sems.at[b + 1]),
            pltpu.make_async_copy(wut_hbm.at[pl.ds(0, FM), :],
                                  wgu_v.at[pl.ds(FM, FM), :], sems.at[b + 2]),
            pltpu.make_async_copy(wgt_hbm.at[pl.ds(FM, FT), :],
                                  wgu_v.at[pl.ds(2 * FM, FT), :],
                                  sems.at[b + 3]),
            pltpu.make_async_copy(wut_hbm.at[pl.ds(FM, FT), :],
                                  wgu_v.at[pl.ds(2 * FM + FT, FT), :],
                                  sems.at[b + 4]),
            pltpu.make_async_copy(wd_hbm, wd_v, sems.at[b + 5]),
        ]

    rowv = lax.broadcasted_iota(jnp.int32, (_VR, TQ), 0)
    row8 = lax.broadcasted_iota(jnp.int32, (8, TQ), 0)
    row8l = lax.broadcasted_iota(jnp.int32, (8, _LANES), 0)

    def scores_mxu(h, qb, c, par, salt, s_dst, mrun):
        n = KC - 16 if c in vchunks else KC
        z = pl.multiple_of(opaque_zero(h, 600 + salt) * 8, 8)
        kc = pltpu.bitcast(
            kh_scr[par][pl.ds(z + c * KC // 2, n // 2), :], bf16)
        st = jnp.dot(kc[:, 0:32], pltpu.bitcast(qm_scr[qb, h], bf16),
                     preferred_element_type=f32)
        s_dst[c * KC:c * KC + n, :] = st
        cm = jnp.max(st.reshape(n // 8, 8, TQ), axis=0)
        return ((cm if mrun is None else jnp.maximum(mrun, cm)),
                [st[r:r + 8, :] for r in _TE], [st[r:r + 8, :] for r in _TV])

    def scores_vpu(h, qb, g, kb_ref, s_dst, mrun, start, salt):
        z = 0 if salt is None else opaque_zero(h, salt)
        hq = h + opaque_zero(h, 100 + g % 4)
        acc = [None] * NJ
        for d in range(DH):
            if d % 2 == 0:
                kb2 = kb_ref[pl.ds(z + (g * DH + d), 2)]
            kb = kb2[d % 2]
            for j in range(NJ):
                t = kb * qf_scr[qb, hq, d:d + 1, j * _LANES:(j + 1) * _LANES]
                if acc[j] is None and start is not None:
                    t = jnp.where(row8l < opaque_zero(h, 300),
                                  start[:, j * _LANES:(j + 1) * _LANES], t)
                acc[j] = t if acc[j] is None else acc[j] + t
        st = jnp.concatenate(acc, axis=1)
        s_dst[vrow[g]:vrow[g] + 8, :] = st
        return (st if mrun is None else jnp.maximum(mrun, st)), st

    def build_kb(h, d, kb_ref, start=None):
        red = None
        for i in range(n16):
            kw = kv_scr[h, i * 8:(i + 1) * 8, :]
            if start is not None:
                kw = jnp.where(row8l < opaque_zero(h, 301),
                               pltpu.bitcast(start[:, 0:_LANES], u32), kw)
            b = jnp.broadcast_to(kw[:, d:d + 1], (8, _LANES))
            bf = pltpu.bitcast(b, bf16).astype(f32)
            kb_ref[(2 * i) * DH + d] = bf[0:8]
            kb_ref[(2 * i + 1) * DH + d] = bf[8:16]
            red = b if red is None else red | b
        red = pltpu.bitcast(red, f32)
        return jnp.concatenate([red] * NJ, axis=1)

    def build_kh(h, i, kh_ref, start=None):
        shift = (_LANES - (h % HPS) * DH) % _LANES
        red = None
        for a in range(8):
            r = i * 64 + a * 8
            kw = k_scr[h // HPS, r:r + 8, :]
            if start is not None:
                kw = jnp.where(row8l < opaque_zero(h, 302),
                               pltpu.bitcast(start[:, 0:_LANES], u32), kw)
            b = pltpu.roll(kw, shift, 1)
            kh_ref[r:r + 8, :] = b
            red = b if red is None else red | b
        red = pltpu.bitcast(red, f32)
        return jnp.concatenate([red] * NJ, axis=1)

    def pv_chunk(h, c, s_src, m, acc, tie):
        z = pl.multiple_of(opaque_zero(h, 0) * KC, KC)
        sv = s_src[pl.ds(z + c * KC, KC), :].reshape(KC // 8, 8, TQ)
        ps = []
        for hf in (1, 0):
            mh = m
            for i, t in enumerate(tie[hf] if tie is not None else ()):
                mh = jnp.where(row8 < opaque_zero(h, 200 + i), t, mh)
            lo = 0 if hf == 1 else KC // 16
            ps.append(jnp.exp2(sv[lo:lo + KC // 16] - mh[None]))
        p = jnp.concatenate(ps, axis=0).reshape(KC, TQ)
        o = lax.dot_general(vx_scr[h, :, c * KC:(c + 1) * KC], p, _NN,
                            preferred_element_type=f32)
        return o if acc is None else o + acc

    def finish(h, qb, o):
        off = (DH * h) % 8
        w0 = pl.multiple_of(DH * h - off, 8)
        l = jnp.where(off == 0, o[_VR - 1:_VR, :], o[0:1, :])
        on = o * (1.0 / l)
        valid = (rowv >= off) & (rowv < off + DH)
        pltpu.store(ot_scr.at[qb, pl.ds(w0, _VR), :], on, mask=valid)

    def score_unit(h, qb, par, salt, gstate, pre_build=False):
        s_dst = s_scr[qb]
        kb_ref = kb_scr[par]
        state = {"mrun": None, "mv": None}
        slots = []
        gdone = 0
        bdone = 0
        for c in range(NC):
            gs, bs = [], []
            for hf in range(2):
                while gdone < NG and gdone * 2 * NC < (2 * c + hf + 1) * NG:
                    while pre_build and bdone < DH:
                        bs.append(bdone)
                        bdone += 1
                    gs.append((gdone, hf))
                    gdone += 1

            def run(c=c, gs=tuple(gs), bs=tuple(bs)):
                if pre_build:
                    for i in ((0, 1) if c == 0 else (c + 1,)):
                        if i < S // 128:
                            build_kh(h, i, kh_scr[par])
                state["mrun"], te, mid = scores_mxu(
                    h, qb, c, par, salt or 0, s_dst, state["mrun"])
                tie = [[te[0]], [te[1]]]
                start = gstate.get("mid", (None, None))
                gstate["mid"] = mid
                for g in bs:
                    build_kb(h, g, kb_ref)
                for g, hf in gs:
                    state["mv"], vt = scores_vpu(
                        h, qb, g, kb_ref, s_dst, state["mv"], start[hf], salt)
                    tie[hf].append(vt)
                for hf, v in gstate.pop("late", ()):
                    tie[hf].append(v)
                t = gstate["t"] = gstate.get("t", -1) + 1
                for (fn, bh, g, bref) in gstate.get("builds", {}).get(t, ()):
                    gstate.setdefault("late", []).append(
                        (g % 2, fn(bh, g, bref, start[0])))
                return tie
            slots.append(run)

        def final():
            mm = state["mrun"]
            if state["mv"] is not None:
                mm = jnp.maximum(mm, state["mv"])
            return jnp.broadcast_to(
                jnp.max(mm, axis=0, keepdims=True), (8, TQ))
        return slots, final

    @pl.when(step == 0)
    def _():
        wc = w_copies()
        x_copy(0).start()
        wc[0].start()
        if _DM == 0:
            for c in range(1, NQ):
                x_copy(c).start()
            wc[1].start()
            wc[2].start()

        s_scr[NQ - 2][(NC - _LP) * KC:, :] = jnp.zeros((_LP * KC, TQ), f32)
        s_scr[NQ - 1][...] = jnp.zeros((S, TQ), f32)

        def ln1(c, i):
            r = pl.multiple_of(c * TQ + i * _LNR, _LNR)
            xn_scr[pl.ds(r, _LNR), :] = _layernorm_f32(
                x_v[pl.ds(r, _LNR), :].astype(f32)).astype(bf16)

        x_copy(0).wait()
        if _DM == 1:
            x_copy(1).start()
        for i in range(TQ // _LNR):
            ln1(0, i)
        wc[0].wait()
        if _DM == 1:
            for c in range(2, NQ):
                x_copy(c).start()
            wc[1].start()
            wc[2].start()

        def kproj(c, carry, last=False):
            if not last:
                x_copy(c + 1).wait()
            nk = TQ // _KM
            assert _KM == KC
            order = vloc + [i for i in range(nk) if i not in vloc]
            for n, i in enumerate(order):
                r = pl.multiple_of(c * TQ + i * _KM, _KM)
                k = jnp.dot(xn_scr[pl.ds(r, _KM), :], wk_v[...],
                            preferred_element_type=f32).astype(bf16)
                r2 = pl.multiple_of((c * TQ + i * _KM) // 2, _KM // 2)
                for s in range(NSLAB):
                    a = s * HPS * DH
                    if a + _LANES <= D:
                        blk = k[:, a:a + _LANES]
                    else:
                        blk = jnp.concatenate(
                            [k[:, a:], jnp.zeros((_KM, a + _LANES - D), bf16)],
                            axis=1)
                    k_scr[s, pl.ds(r2, _KM // 2), :] = pltpu.bitcast(blk, u32)
                    if s == 0:
                        kh_scr[0][pl.ds(r2, _KM // 2), :] = (
                            pltpu.bitcast(blk, u32))
                if i in vloc:
                    kt = jnp.concatenate(
                        [pltpu.bitcast(k[KC - 16:, :], u32),
                         jnp.zeros((8, _LANES), u32)], axis=1)
                    rk = pl.multiple_of((c * len(vloc) + n) * 8, 8)
                    for h in range(_H):
                        kv_scr[h, pl.ds(rk, 8), :] = (
                            kt[:, h * DH:h * DH + _LANES])
                nl = (TQ // _LNR) // nk
                for ii in range(n * nl, (n + 1) * nl):
                    if not last:
                        ln1(c + 1, ii)
                if last and n == len(vloc) - 1:
                    for d in range(DH):
                        build_kb(step, d, kb_scr[0])
            return carry

        lax.fori_loop(0, NQ - 1, kproj, 0)
        kproj(NQ - 1, 0, True)
        wc[1].wait()
        wc[2].wait()
        for cp in late_copies():
            cp.start()

        row32 = lax.broadcasted_iota(jnp.int32, (32, TQ), 0)

        def qvproj(c, carry):
            r0 = pl.multiple_of(c * TQ, TQ)
            qv = jnp.dot(xn_scr[pl.ds(r0, TQ), :], wqv_v[...],
                         preferred_element_type=f32)
            qvt = qv.T
            vt = qvt[D:, :]
            qs = (qvt[0:D + 32, :] * qscale).astype(bf16).astype(f32)
            for h in range(_H):
                w = qs[h * DH:h * DH + 32, :]
                qm_scr[c, h] = pltpu.bitcast(
                    jnp.where(row32 < DH, w, 0.0).astype(bf16), u32)
                if NG:
                    qf_scr[c, h] = w[0:_VR, :]
                w0 = 8 * ((DH * h) // 8)
                ones_row = _VR - 1 if (DH * h) % 8 == 0 else 0
                win = jnp.where(rowv == ones_row, 1.0, vt[w0:w0 + _VR, :])
                vx_scr[h, :, pl.ds(r0, TQ)] = win
            return carry

        lax.fori_loop(0, NQ, qvproj, 0)

        NP = _HU * NQ

        def body(it, carry):
            h0 = it * _HU
            head = lambda u: jnp.clip(h0 + u // NQ, 0, _H - 1)
            ms = {-2: carry[0], -1: carry[2]}
            accs = {-2: carry[1]}
            builds = {}
            for i in range(_HU):
                t0 = i * NQ * NC + 1
                t1 = (i + 1) * NQ * NC - 3
                items = [(build_kh, g, kh_scr[(i + 1) % 2])
                         for g in range(S // 128)]
                items += [(build_kb, g, kb_scr[(i + 1) % 2])
                          for g in range(DH if NG else 0)]
                for n, (fn, g, ref) in enumerate(items):
                    t = t0 + (n * (t1 - t0)) // len(items)
                    builds.setdefault(t, []).append(
                        (fn, head((i + 1) * NQ), g, ref))
            gstate = {"builds": builds}
            tie = None
            for u in range(NP):
                slots, final = score_unit(
                    head(u), u % NQ, (u // NQ) % 2, u, gstate)
                for c in range(NC):
                    new_tie = slots[c]()
                    p = (u - 1) * NC + c - _LP
                    pu, pc = p // NC, p % NC
                    accs[pu] = pv_chunk(head(pu), pc, s_scr[pu % NQ], ms[pu],
                                        accs.get(pu), tie)
                    if pc == NC - 1:
                        finish(head(pu), pu % NQ, accs[pu])
                    tie = new_tie
                ms[u] = final()
            return ms[NP - 2], accs[NP - 2], ms[NP - 1]

        m2, acc2, m3 = lax.fori_loop(
            0, _H // _HU, body,
            (jnp.zeros((8, TQ), f32), jnp.zeros((_VR, TQ), f32),
             jnp.zeros((8, TQ), f32)))
        hl = _H - 1 + step
        for pc in range(NC - _LP, NC):
            acc2 = pv_chunk(hl, pc, s_scr[NQ - 2], m2, acc2, None)
        finish(hl, NQ - 2, acc2)
        acc3 = None
        for pc in range(NC):
            acc3 = pv_chunk(hl, pc, s_scr[NQ - 1], m3, acc3, None)
        finish(hl, NQ - 1, acc3)
        for cp in late_copies():
            cp.wait()

    R = TQ // _FS
    hres = []
    for r in range(_FS):
        o_nat = ot_scr[step, :, r * R:(r + 1) * R].T.astype(bf16)
        attn = jnp.dot(o_nat, wo_v[...], preferred_element_type=f32)
        q0 = pl.multiple_of(step * TQ + r * R, R)
        hres.append(x_v[pl.ds(q0, R), :].astype(f32) + attn)
    for r in range(_FS):
        hn = _layernorm_f32(hres[r]).astype(bf16)
        gu = lax.dot_general(hn, wgu_v[...], _NT, preferred_element_type=f32)
        g = jnp.concatenate([gu[:, 0:FM], gu[:, 2 * FM:2 * FM + FT]], axis=1)
        u = jnp.concatenate([gu[:, FM:2 * FM], gu[:, 2 * FM + FT:]], axis=1)
        act = (g * jax.nn.sigmoid(g) * u).astype(bf16)
        dn = jnp.dot(act, wd_v[...], preferred_element_type=f32)
        o_ref[r * R:(r + 1) * R, :] = (hres[r] + dn).astype(o_ref.dtype)


@jax.jit
def pallas_sequential_preLN__mha_block__swiglu_ffn__prompt_kernel(
    A_x: jax.Array,
    A_wqkv: jax.Array,
    A_wo: jax.Array,
    B_x: jax.Array,
    B_w_gate: jax.Array,
    B_w_up: jax.Array,
    B_w_down: jax.Array,
):
    del B_x
    B, S, D = A_x.shape
    assert B == 1
    F = B_w_gate.shape[1]
    DH = D // _H
    HPS = _LANES // DH
    NSLAB = -(-_H // HPS)
    NQ = S // _TQ
    x = A_x.reshape(S, D)
    bf16 = jnp.bfloat16
    f32 = jnp.float32
    nkb = max(_NV // 8, 1) * DH

    kern = functools.partial(_kernel, S=S, D=D, F=F, DH=DH, HPS=HPS,
                             NSLAB=NSLAB)
    out = pl.pallas_call(
        kern,
        grid=(NQ,),
        in_specs=[pl.BlockSpec(memory_space=pl.ANY)] * 6,
        out_specs=pl.BlockSpec((_TQ, D), lambda i: (i, 0)),
        out_shape=jax.ShapeDtypeStruct((S, D), A_x.dtype),
        scratch_shapes=[
            pltpu.VMEM((S, D), bf16),
            pltpu.VMEM((D, D), bf16),
            pltpu.VMEM((D, 2 * D), bf16),
            pltpu.VMEM((D, D), bf16),
            pltpu.VMEM((2 * F, D), bf16),
            pltpu.VMEM((F, D), bf16),
            pltpu.VMEM((S, D), bf16),
            pltpu.VMEM((NQ, _H, 16, _TQ), jnp.uint32),
            pltpu.VMEM((NSLAB, S // 2, _LANES), jnp.uint32),
            pltpu.VMEM((_H, _VR, S), f32),
            pltpu.VMEM((NQ, D, _TQ), f32),
            pltpu.VMEM((S, _TQ), f32),
            pltpu.VMEM((S, _TQ), f32),
            pltpu.VMEM((S, _TQ), f32),
            pltpu.VMEM((S, _TQ), f32),
            pltpu.VMEM((_H, max(_NV // 2, 8), _LANES), jnp.uint32),
            pltpu.VMEM((NQ, _H, _VR, _TQ), f32),
            pltpu.VMEM((nkb, 8, _LANES), f32),
            pltpu.VMEM((nkb, 8, _LANES), f32),
            pltpu.VMEM((S // 2, _LANES), jnp.uint32),
            pltpu.VMEM((S // 2, _LANES), jnp.uint32),
            pltpu.SemaphoreType.DMA((NQ + 9,)),
        ],
        compiler_params=pltpu.CompilerParams(
            dimension_semantics=("arbitrary",),
            vmem_limit_bytes=110 * 1024 * 1024,
        ),
    )(x, A_wqkv, A_wo, B_w_gate.T, B_w_up.T, B_w_down)
    return out.reshape(B, S, D)
```

```python
import functools
import math

import jax
import jax.numpy as jnp
from jax import lax
import jax.experimental.pallas as pl
import jax.experimental.pallas.tpu as pltpu

_H = 32
_EPS = 1e-5
_LANES = 128
_TQ = 512
_KC = 128
_VR = 24
_VL = ((0, 1, 3), (1,))
_FS = 2
_HU = 2
_LP = 2
_TE = (0, 48)
_TV = (48, 104)
_KM = 128
_DM = 1
_KS = 2
_LNR = 64

_NN = (((1,), (0,)), ((), ()))
_NT = (((1,), (1,)), ((), ()))


def _layernorm_f32(x):
    m = jnp.mean(x, axis=-1, keepdims=True)
    xc = x - m
    v = jnp.mean(xc * xc, axis=-1, keepdims=True)
    return xc * lax.rsqrt(v + _EPS)


def _kernel(x_hbm, wqkv_hbm, wo_hbm, wgt_hbm, wut_hbm, wd_hbm, o_ref,
            x_v, wk_v, wqv_v, wo_v, wgu_v, wd_v,
            xn_scr, qm_scr, k_scr, vx_scr, ot_scr,
            s0_scr, s1_scr, s2_scr, s3_scr,
            kv_scr, qf_scr, kb0_scr, kb1_scr, kh0_scr, kh1_scr, sems,
            *, S, D, F, DH, HPS, NSLAB):
    step = pl.program_id(0)
    s_scr = (s0_scr, s1_scr, s2_scr, s3_scr)
    kb_scr = (kb0_scr, kb1_scr)
    kh_scr = (kh0_scr, kh1_scr)
    qscale = (DH ** -0.5) * math.log2(math.e)
    TQ, KC = _TQ, _KC
    NC = S // KC
    NQ = S // TQ
    NJ = TQ // _LANES
    FM = (F // _LANES) * _LANES
    FT = F - FM
    bf16 = jnp.bfloat16
    f32 = jnp.float32
    u32 = jnp.uint32
    CPB = TQ // KC
    vchunks = ([b * CPB + v for b in range(NQ - 1) for v in _VL[0]]
               + [(NQ - 1) * CPB + v for v in _VL[1]])
    n16 = len(vchunks)
    NG = 2 * n16
    vrow = [vc * KC + KC - 16 + o for vc in vchunks for o in (0, 8)]

    def opaque_zero(h, salt):
        return lax.shift_right_logical(h + salt, 10)

    def x_copy(c):
        return pltpu.make_async_copy(
            x_hbm.at[pl.ds(c * TQ, TQ), :], x_v.at[pl.ds(c * TQ, TQ), :],
            sems.at[c])

    def w_copies():
        return [
            pltpu.make_async_copy(wqkv_hbm.at[:, pl.ds(D, D)], wk_v,
                                  sems.at[NQ]),
            pltpu.make_async_copy(wqkv_hbm.at[:, pl.ds(0, D)],
                                  wqv_v.at[:, pl.ds(0, D)], sems.at[NQ + 1]),
            pltpu.make_async_copy(wqkv_hbm.at[:, pl.ds(2 * D, D)],
                                  wqv_v.at[:, pl.ds(D, D)], sems.at[NQ + 2]),
        ]

    def late_copies():
        b = NQ + 3
        return [
            pltpu.make_async_copy(wo_hbm, wo_v, sems.at[b]),
            pltpu.make_async_copy(wgt_hbm.at[pl.ds(0, FM), :],
                                  wgu_v.at[pl.ds(0, FM), :], sems.at[b + 1]),
            pltpu.make_async_copy(wut_hbm.at[pl.ds(0, FM), :],
                                  wgu_v.at[pl.ds(FM, FM), :], sems.at[b + 2]),
            pltpu.make_async_copy(wgt_hbm.at[pl.ds(FM, FT), :],
                                  wgu_v.at[pl.ds(2 * FM, FT), :],
                                  sems.at[b + 3]),
            pltpu.make_async_copy(wut_hbm.at[pl.ds(FM, FT), :],
                                  wgu_v.at[pl.ds(2 * FM + FT, FT), :],
                                  sems.at[b + 4]),
            pltpu.make_async_copy(wd_hbm, wd_v, sems.at[b + 5]),
        ]

    rowv = lax.broadcasted_iota(jnp.int32, (_VR, TQ), 0)
    row8 = lax.broadcasted_iota(jnp.int32, (8, TQ), 0)
    row8l = lax.broadcasted_iota(jnp.int32, (8, _LANES), 0)

    def never(i):
        return row8l < opaque_zero(step, 200 + i)

    def tiles(v):
        return [v[:, j * _LANES:(j + 1) * _LANES] for j in range(NJ)]

    def scores_mxu(h, qb, c, par, salt, s_dst, mrun):
        n = KC - 16 if c in vchunks else KC
        z = pl.multiple_of(opaque_zero(h, 600 + salt) * 8, 8)
        kc = pltpu.bitcast(
            kh_scr[par][pl.ds(z + c * KC // 2, n // 2), :], bf16)
        st = jnp.dot(kc[:, 0:32], pltpu.bitcast(qm_scr[qb, h], bf16),
                     preferred_element_type=f32)
        s_dst[c * KC:c * KC + n, :] = st
        cm = jnp.max(st.reshape(n // 8, 8, TQ), axis=0)
        return ((cm if mrun is None else jnp.maximum(mrun, cm)),
                [tiles(st[r:r + 8, :]) for r in _TE],
                [tiles(st[r:r + 8, :]) for r in _TV])

    def scores_vpu(h, qb, g, js, kb_ref, s_dst, start, salt):
        hq = h + opaque_zero(h, 100 + g % 4)
        acc = {}
        for i0 in range(0, len(js), _KS):
            z = opaque_zero(h, 700 + salt * NJ + js[i0])
            for d in range(DH):
                kb = kb_ref[z + (g * DH + d)]
                for j in js[i0:i0 + _KS]:
                    t = kb * qf_scr[qb, hq, d:d + 1,
                                    j * _LANES:(j + 1) * _LANES]
                    if j not in acc and start is not None:
                        t = jnp.where(never(0), start[j], t)
                    acc[j] = acc[j] + t if j in acc else t
        for j in js:
            s_dst[vrow[g]:vrow[g] + 8, j * _LANES:(j + 1) * _LANES] = acc[j]
        return acc

    def build_kb(h, d, kb_ref, start=None):
        red = None
        for i in range(n16):
            kw = kv_scr[h, i * 8:(i + 1) * 8, :]
            if start is not None:
                kw = jnp.where(never(0), pltpu.bitcast(start[0], u32), kw)
            b = jnp.broadcast_to(kw[:, d:d + 1], (8, _LANES))
            bf = pltpu.bitcast(b, bf16).astype(f32)
            kb_ref[(2 * i) * DH + d] = bf[0:8]
            kb_ref[(2 * i + 1) * DH + d] = bf[8:16]
            red = b if red is None else red | b
        return pltpu.bitcast(red, f32)

    def build_kh(h, i, kh_ref, start=None):
        shift = (_LANES - (h % HPS) * DH) % _LANES
        red = None
        for a in range(8):
            r = i * 64 + a * 8
            kw = k_scr[h // HPS, r:r + 8, :]
            if start is not None:
                kw = jnp.where(never(0), pltpu.bitcast(start[0], u32), kw)
            b = pltpu.roll(kw, shift, 1)
            kh_ref[r:r + 8, :] = b
            red = b if red is None else red | b
        return pltpu.bitcast(red, f32)

    def pv_chunk(h, c, s_src, m, acc, tie):
        z = pl.multiple_of(opaque_zero(h, 0) * KC, KC)
        sv = s_src[pl.ds(z + c * KC, KC), :].reshape(KC // 8, 8, TQ)
        ps = []
        for hf in (1, 0):
            mh = tiles(m)
            for j in range(NJ if tie is not None else 0):
                for i, t in enumerate(tie[hf][j]):
                    mh[j] = jnp.where(never(i), t, mh[j])
            mh = jnp.concatenate(mh, axis=1)
            lo = 0 if hf == 1 else KC // 16
            ps.append(jnp.exp2(sv[lo:lo + KC // 16] - mh[None]))
        p = jnp.concatenate(ps, axis=0).reshape(KC, TQ)
        o = lax.dot_general(vx_scr[h, :, c * KC:(c + 1) * KC], p, _NN,
                            preferred_element_type=f32)
        return o if acc is None else o + acc

    def finish(h, qb, o):
        off = (DH * h) % 8
        w0 = pl.multiple_of(DH * h - off, 8)
        l = jnp.where(off == 0, o[_VR - 1:_VR, :], o[0:1, :])
        on = o * (1.0 / l)
        valid = (rowv >= off) & (rowv < off + DH)
        pltpu.store(ot_scr.at[qb, pl.ds(w0, _VR), :], on, mask=valid)

    def score_unit(h, qb, par, salt, gstate):
        s_dst = s_scr[qb]
        kb_ref = kb_scr[par]
        state = {"mrun": None, "mv": {}}
        assert NG >= NC and ((NG - NC) * NJ) % NC == 0
        nb = ((NG - NC) * NJ) // NC
        extra = [(g, j) for g in range(NC, NG) for j in range(NJ)]
        slots = []
        for c in range(NC):
            gs = [(c, tuple(range(NJ)), 0)]
            mine = extra[c * nb:(c + 1) * nb]
            for g in sorted(set(g for g, _ in mine)):
                gs.append((g, tuple(j for gg, j in mine if gg == g), 1))

            def run(c=c, gs=tuple(gs)):
                state["mrun"], te, mid = scores_mxu(
                    h, qb, c, par, salt, s_dst, state["mrun"])
                tie = [[[te[hf][j]] for j in range(NJ)] for hf in range(2)]
                start = gstate.get("mid", (None, None))
                gstate["mid"] = mid
                for g, js, hf in gs:
                    acc = scores_vpu(h, qb, g, js, kb_ref, s_dst, start[hf],
                                     salt)
                    for j, v in acc.items():
                        tie[hf][j].append(v)
                        mv = state["mv"]
                        mv[j] = jnp.maximum(mv[j], v) if j in mv else v
                for hf, j, v in gstate.pop("late", ()):
                    tie[hf][j].append(v)
                t = gstate["t"] = gstate.get("t", -1) + 1
                for (fn, bh, g, bref) in gstate.get("builds", {}).get(t, ()):
                    gstate.setdefault("late", []).append(
                        (g % 2, g % NJ, fn(bh, g, bref, start[0])))
                return tie
            slots.append(run)

        def final():
            mm = jnp.maximum(
                state["mrun"],
                jnp.concatenate([state["mv"][j] for j in range(NJ)], axis=1))
            return jnp.broadcast_to(
                jnp.max(mm, axis=0, keepdims=True), (8, TQ))
        return slots, final

    @pl.when(step == 0)
    def _():
        wc = w_copies()
        x_copy(0).start()
        wc[0].start()
        if _DM == 0:
            for c in range(1, NQ):
                x_copy(c).start()
            wc[1].start()
            wc[2].start()

        s_scr[NQ - 2][(NC - _LP) * KC:, :] = jnp.zeros((_LP * KC, TQ), f32)
        s_scr[NQ - 1][...] = jnp.zeros((S, TQ), f32)

        def ln1(c, i):
            r = pl.multiple_of(c * TQ + i * _LNR, _LNR)
            xn_scr[pl.ds(r, _LNR), :] = _layernorm_f32(
                x_v[pl.ds(r, _LNR), :].astype(f32)).astype(bf16)

        x_copy(0).wait()
        if _DM == 1:
            x_copy(1).start()
        for i in range(TQ // _LNR):
            ln1(0, i)
        wc[0].wait()
        if _DM == 1:
            for c in range(2, NQ):
                x_copy(c).start()
            wc[1].start()
            wc[2].start()

        def kproj(c, carry, last=False):
            if not last:
                x_copy(c + 1).wait()
            nk = TQ // _KM
            assert _KM == KC
            vloc = list(_VL[1 if last else 0])
            order = vloc + [i for i in range(nk) if i not in vloc]
            for n, i in enumerate(order):
                r = pl.multiple_of(c * TQ + i * _KM, _KM)
                k = jnp.dot(xn_scr[pl.ds(r, _KM), :], wk_v[...],
                            preferred_element_type=f32).astype(bf16)
                r2 = pl.multiple_of((c * TQ + i * _KM) // 2, _KM // 2)
                for s in range(NSLAB):
                    a = s * HPS * DH
                    if a + _LANES <= D:
                        blk = k[:, a:a + _LANES]
                    else:
                        blk = jnp.concatenate(
                            [k[:, a:], jnp.zeros((_KM, a + _LANES - D), bf16)],
                            axis=1)
                    k_scr[s, pl.ds(r2, _KM // 2), :] = pltpu.bitcast(blk, u32)
                    if s == 0:
                        kh_scr[0][pl.ds(r2, _KM // 2), :] = (
                            pltpu.bitcast(blk, u32))
                if i in vloc:
                    kt = jnp.concatenate(
                        [pltpu.bitcast(k[KC - 16:, :], u32),
                         jnp.zeros((8, _LANES), u32)], axis=1)
                    rk = pl.multiple_of((c * len(_VL[0]) + n) * 8, 8)
                    for h in range(_H):
                        kv_scr[h, pl.ds(rk, 8), :] = (
                            kt[:, h * DH:h * DH + _LANES])
                nl = (TQ // _LNR) // nk
                for ii in range(n * nl, (n + 1) * nl):
                    if not last:
                        ln1(c + 1, ii)
                if last and n == len(vloc) - 1:
                    for d in range(DH):
                        build_kb(step, d, kb_scr[0])
            return carry

        lax.fori_loop(0, NQ - 1, kproj, 0)
        kproj(NQ - 1, 0, True)
        wc[1].wait()
        wc[2].wait()
        for cp in late_copies():
            cp.start()

        row32 = lax.broadcasted_iota(jnp.int32, (32, TQ), 0)

        def qvproj(c, carry):
            r0 = pl.multiple_of(c * TQ, TQ)
            qv = jnp.dot(xn_scr[pl.ds(r0, TQ), :], wqv_v[...],
                         preferred_element_type=f32)
            qvt = qv.T
            vt = qvt[D:, :]
            qs = (qvt[0:D + 32, :] * qscale).astype(bf16).astype(f32)
            for h in range(_H):
                w = qs[h * DH:h * DH + 32, :]
                qm_scr[c, h] = pltpu.bitcast(
                    jnp.where(row32 < DH, w, 0.0).astype(bf16), u32)
                if NG:
                    qf_scr[c, h] = w[0:_VR, :]
                w0 = 8 * ((DH * h) // 8)
                ones_row = _VR - 1 if (DH * h) % 8 == 0 else 0
                win = jnp.where(rowv == ones_row, 1.0, vt[w0:w0 + _VR, :])
                vx_scr[h, :, pl.ds(r0, TQ)] = win
            return carry

        lax.fori_loop(0, NQ, qvproj, 0)

        NP = _HU * NQ

        def body(it, carry):
            h0 = it * _HU
            head = lambda u: jnp.clip(h0 + u // NQ, 0, _H - 1)
            ms = {-2: carry[0], -1: carry[2]}
            accs = {-2: carry[1]}
            builds = {}
            for i in range(_HU):
                t0 = i * NQ * NC + 1
                t1 = (i + 1) * NQ * NC - 3
                items = [(build_kh, g, kh_scr[(i + 1) % 2])
                         for g in range(S // 128)]
                items += [(build_kb, g, kb_scr[(i + 1) % 2])
                          for g in range(DH if NG else 0)]
                for n, (fn, g, ref) in enumerate(items):
                    t = t0 + (n * (t1 - t0)) // len(items)
                    builds.setdefault(t, []).append(
                        (fn, head((i + 1) * NQ), g, ref))
            gstate = {"builds": builds}
            tie = None
            for u in range(NP):
                slots, final = score_unit(
                    head(u), u % NQ, (u // NQ) % 2, u, gstate)
                for c in range(NC):
                    new_tie = slots[c]()
                    p = (u - 1) * NC + c - _LP
                    pu, pc = p // NC, p % NC
                    accs[pu] = pv_chunk(head(pu), pc, s_scr[pu % NQ], ms[pu],
                                        accs.get(pu), tie)
                    if pc == NC - 1:
                        finish(head(pu), pu % NQ, accs[pu])
                    tie = new_tie
                ms[u] = final()
            return ms[NP - 2], accs[NP - 2], ms[NP - 1]

        m2, acc2, m3 = lax.fori_loop(
            0, _H // _HU, body,
            (jnp.zeros((8, TQ), f32), jnp.zeros((_VR, TQ), f32),
             jnp.zeros((8, TQ), f32)))
        hl = _H - 1 + step
        for pc in range(NC - _LP, NC):
            acc2 = pv_chunk(hl, pc, s_scr[NQ - 2], m2, acc2, None)
        finish(hl, NQ - 2, acc2)
        acc3 = None
        for pc in range(NC):
            acc3 = pv_chunk(hl, pc, s_scr[NQ - 1], m3, acc3, None)
        finish(hl, NQ - 1, acc3)
        for cp in late_copies():
            cp.wait()

    R = TQ // _FS
    hres = []
    for r in range(_FS):
        o_nat = ot_scr[step, :, r * R:(r + 1) * R].T.astype(bf16)
        attn = jnp.dot(o_nat, wo_v[...], preferred_element_type=f32)
        q0 = pl.multiple_of(step * TQ + r * R, R)
        hres.append(x_v[pl.ds(q0, R), :].astype(f32) + attn)
    for r in range(_FS):
        hn = _layernorm_f32(hres[r]).astype(bf16)
        gu = lax.dot_general(hn, wgu_v[...], _NT, preferred_element_type=f32)
        g = jnp.concatenate([gu[:, 0:FM], gu[:, 2 * FM:2 * FM + FT]], axis=1)
        u = jnp.concatenate([gu[:, FM:2 * FM], gu[:, 2 * FM + FT:]], axis=1)
        act = (g * jax.nn.sigmoid(g) * u).astype(bf16)
        dn = jnp.dot(act, wd_v[...], preferred_element_type=f32)
        o_ref[r * R:(r + 1) * R, :] = (hres[r] + dn).astype(o_ref.dtype)


@jax.jit
def pallas_sequential_preLN__mha_block__swiglu_ffn__prompt_kernel(
    A_x: jax.Array,
    A_wqkv: jax.Array,
    A_wo: jax.Array,
    B_x: jax.Array,
    B_w_gate: jax.Array,
    B_w_up: jax.Array,
    B_w_down: jax.Array,
):
    del B_x
    B, S, D = A_x.shape
    assert B == 1
    F = B_w_gate.shape[1]
    DH = D // _H
    HPS = _LANES // DH
    NSLAB = -(-_H // HPS)
    NQ = S // _TQ
    x = A_x.reshape(S, D)
    bf16 = jnp.bfloat16
    f32 = jnp.float32
    n16 = (NQ - 1) * len(_VL[0]) + len(_VL[1])
    nkb = 2 * n16 * DH

    kern = functools.partial(_kernel, S=S, D=D, F=F, DH=DH, HPS=HPS,
                             NSLAB=NSLAB)
    out = pl.pallas_call(
        kern,
        grid=(NQ,),
        in_specs=[pl.BlockSpec(memory_space=pl.ANY)] * 6,
        out_specs=pl.BlockSpec((_TQ, D), lambda i: (i, 0)),
        out_shape=jax.ShapeDtypeStruct((S, D), A_x.dtype),
        scratch_shapes=[
            pltpu.VMEM((S, D), bf16),
            pltpu.VMEM((D, D), bf16),
            pltpu.VMEM((D, 2 * D), bf16),
            pltpu.VMEM((D, D), bf16),
            pltpu.VMEM((2 * F, D), bf16),
            pltpu.VMEM((F, D), bf16),
            pltpu.VMEM((S, D), bf16),
            pltpu.VMEM((NQ, _H, 16, _TQ), jnp.uint32),
            pltpu.VMEM((NSLAB, S // 2, _LANES), jnp.uint32),
            pltpu.VMEM((_H, _VR, S), f32),
            pltpu.VMEM((NQ, D, _TQ), f32),
            pltpu.VMEM((S, _TQ), f32),
            pltpu.VMEM((S, _TQ), f32),
            pltpu.VMEM((S, _TQ), f32),
            pltpu.VMEM((S, _TQ), f32),
            pltpu.VMEM((_H, 8 * n16, _LANES), jnp.uint32),
            pltpu.VMEM((NQ, _H, _VR, _TQ), f32),
            pltpu.VMEM((nkb, 8, _LANES), f32),
            pltpu.VMEM((nkb, 8, _LANES), f32),
            pltpu.VMEM((S // 2, _LANES), jnp.uint32),
            pltpu.VMEM((S // 2, _LANES), jnp.uint32),
            pltpu.SemaphoreType.DMA((NQ + 9,)),
        ],
        compiler_params=pltpu.CompilerParams(
            dimension_semantics=("arbitrary",),
            vmem_limit_bytes=110 * 1024 * 1024,
        ),
    )(x, A_wqkv, A_wo, B_w_gate.T, B_w_up.T, B_w_down)
    return out.reshape(B, S, D)
```

```python
import functools
import math

import jax
import jax.numpy as jnp
from jax import lax
import jax.experimental.pallas as pl
import jax.experimental.pallas.tpu as pltpu

_H = 32
_EPS = 1e-5
_LANES = 128
_TQ = 512
_KC = 128
_VR = 24
_NT4 = 8
_FS = 4
_HU = 2
_LQ = 5
_ES = 6
_TV = (48, 104)
_KS = 2
_TE = (16, 72)
_BS = 1
_BR = 1
_BD = 1
_LND = 3
_LNR = 64
_VD = 1
_LMAX = 2.0 ** 40
_LMIN = 2.0 ** -20
_BIG = 3.0e38

_NN = (((1,), (0,)), ((), ()))
_NT = (((1,), (1,)), ((), ()))


def _layernorm_f32(x):
    m = jnp.mean(x, axis=-1, keepdims=True)
    xc = x - m
    v = jnp.mean(xc * xc, axis=-1, keepdims=True)
    return xc * lax.rsqrt(v + _EPS)


def _kernel(x_hbm, wqkv_hbm, wo_hbm, wgt_hbm, wut_hbm, wd_hbm, o_ref,
            x_v, wk_v, wqv_v, wo_v, wgu_v, wd_v,
            xn_scr, qm_scr, k_scr, vx_scr, ot_scr, p0_scr, p1_scr,
            qf_scr, kb0_scr, kb1_scr, kh0_scr, kh1_scr, qc_scr, nc_scr,
            flag_scr, o_v, sems, osems,
            *, S, D, F, DH, HPS, NSLAB):
    step = pl.program_id(0)
    p_scr = (p0_scr, p1_scr)
    kb_scr = (kb0_scr, kb1_scr)
    kh_scr = (kh0_scr, kh1_scr)
    qscale = (DH ** -0.5) * math.log2(math.e)
    TQ, KC = _TQ, _KC
    NC = S // KC
    NQ = S // TQ
    NJ = TQ // _LANES
    FM = (F // _LANES) * _LANES
    FT = F - FM
    bf16 = jnp.bfloat16
    f32 = jnp.float32
    u32 = jnp.uint32
    n16 = (_NT4 * NC) // (2 * NJ)
    vchunks = [c for c in range(NC)
               if ((c + 1) * n16) // NC > (c * n16) // NC]
    assert len(vchunks) == n16
    NG = 2 * n16
    vrow = [vc * KC + KC - 16 + o for vc in vchunks for o in (0, 8)]

    def opaque_zero(h, salt):
        return lax.shift_right_logical(h + salt, 10)

    def x_copy(c):
        return pltpu.make_async_copy(
            x_hbm.at[pl.ds(c * TQ, TQ), :], x_v.at[pl.ds(c * TQ, TQ), :],
            sems.at[c])

    def w_copies():
        return [
            pltpu.make_async_copy(wqkv_hbm.at[:, pl.ds(D, D)], wk_v,
                                  sems.at[NQ]),
            pltpu.make_async_copy(wqkv_hbm.at[:, pl.ds(0, D)],
                                  wqv_v.at[:, pl.ds(0, D)], sems.at[NQ + 1]),
            pltpu.make_async_copy(wqkv_hbm.at[:, pl.ds(2 * D, D)],
                                  wqv_v.at[:, pl.ds(D, D)], sems.at[NQ + 2]),
        ]

    def late_copies():
        b = NQ + 3
        return [
            pltpu.make_async_copy(wo_hbm, wo_v, sems.at[b]),
            pltpu.make_async_copy(wgt_hbm.at[pl.ds(0, FM), :],
                                  wgu_v.at[pl.ds(0, FM), :], sems.at[b + 1]),
            pltpu.make_async_copy(wut_hbm.at[pl.ds(0, FM), :],
                                  wgu_v.at[pl.ds(FM, FM), :], sems.at[b + 2]),
            pltpu.make_async_copy(wgt_hbm.at[pl.ds(FM, FT), :],
                                  wgu_v.at[pl.ds(2 * FM, FT), :],
                                  sems.at[b + 3]),
            pltpu.make_async_copy(wut_hbm.at[pl.ds(FM, FT), :],
                                  wgu_v.at[pl.ds(2 * FM + FT, FT), :],
                                  sems.at[b + 4]),
            pltpu.make_async_copy(wd_hbm, wd_v, sems.at[b + 5]),
        ]

    rowv = lax.broadcasted_iota(jnp.int32, (_VR, TQ), 0)
    row8 = lax.broadcasted_iota(jnp.int32, (8, TQ), 0)
    row8l = lax.broadcasted_iota(jnp.int32, (8, _LANES), 0)

    def never(i):
        return row8l < opaque_zero(step, 200 + i)

    def tiles(v):
        return [v[:, j * _LANES:(j + 1) * _LANES] for j in range(NJ)]

    def with_ones(kw):
        lane = lax.broadcasted_iota(jnp.int32, kw.shape, 1)
        return jnp.where((lane == DH) | (lane == DH + 1),
                         jnp.uint32(0x3F803F80), kw)

    def nrows(c):
        return KC - 16 if c in vchunks else KC

    def qk_dot(h, c, par, salt, w):
        z = pl.multiple_of(opaque_zero(h, 600 + salt) * 8, 8)
        kc = pltpu.bitcast(
            kh_scr[par][pl.ds(z + c * KC // 2, nrows(c) // 2), :], bf16)
        return jnp.dot(kc[:, 0:32], pltpu.bitcast(w, bf16),
                       preferred_element_type=f32)

    def estimate(h, qb, par, salt, sl):
        st = qk_dot(h, 0, par, salt, qm_scr[qb, h])
        p_scr[sl][0:nrows(0), :] = st
        c = jnp.max(jnp.max(st.reshape(nrows(0) // 8, 8, TQ), axis=0),
                    axis=0, keepdims=True)
        hi = c.astype(bf16).astype(f32)
        lo = (c - hi).astype(bf16).astype(f32)
        nc_scr[sl] = jnp.broadcast_to(-(hi + lo), (8, TQ))
        r = DH - 16
        top = jnp.where(row8 < r, qf_scr[qb, h, 16:24, :],
                        jnp.where(row8 == r, -hi,
                                  jnp.where(row8 == r + 1, -lo, 0.0)))
        qc_scr[sl] = pltpu.bitcast(
            jnp.concatenate([top, jnp.zeros((8, TQ), f32)],
                            axis=0).astype(bf16), u32)
        return st

    def probs_mxu(h, qb, c, par, salt, sl):
        w = jnp.concatenate([qm_scr[qb, h, 0:8, :], qc_scr[sl]], axis=0)
        st = qk_dot(h, c, par, salt, w)
        p_scr[sl][c * KC:c * KC + nrows(c), :] = jnp.exp2(st)
        return st

    def probs_vpu(h, qb, g, js, par, sl, start, salt):
        hq = h + opaque_zero(h, 100 + g % 4)
        acc = {}
        for i0 in range(0, len(js), _KS):
            z = opaque_zero(h, 700 + salt * NJ + js[i0])
            for d in range(DH):
                kb = kb_scr[par][z + (g * DH + d)]
                for j in js[i0:i0 + _KS]:
                    t = kb * qf_scr[qb, hq, d:d + 1,
                                    j * _LANES:(j + 1) * _LANES]
                    if j not in acc:
                        acc[j] = nc_scr[sl, :, j * _LANES:(j + 1) * _LANES]
                        if start is not None:
                            acc[j] = jnp.where(never(0), start[j], acc[j])
                    acc[j] = acc[j] + t
        for j in js:
            p_scr[sl][vrow[g]:vrow[g] + 8, j * _LANES:(j + 1) * _LANES] = (
                jnp.exp2(acc[j]))
        return acc

    def build_kb(h, item, par, start=None):
        d, idx = item
        kb_ref = kb_scr[par]
        z = pl.multiple_of(opaque_zero(h, 640 + d) * 8, 8)
        red = None
        for i in idx:
            kw = kh_scr[par][pl.ds(z + vrow[2 * i] // 2, 8), :]
            if start is not None and _BS:
                kw = jnp.where(never(0), pltpu.bitcast(start[0], u32), kw)
            b = jnp.broadcast_to(kw[:, d:d + 1], (8, _LANES))
            bf = pltpu.bitcast(b, bf16).astype(f32)
            kb_ref[(2 * i) * DH + d] = bf[0:8]
            kb_ref[(2 * i + 1) * DH + d] = bf[8:16]
            red = b if (red is None or not _BR) else red | b
        return pltpu.bitcast(red, f32)

    def build_kh(h, rows, par, start=None):
        shift = (_LANES - (h % HPS) * DH) % _LANES
        red = None
        for r in rows:
            kw = k_scr[h // HPS, r:r + 8, :]
            if start is not None and _BS:
                kw = jnp.where(never(0), pltpu.bitcast(start[0], u32), kw)
            b = with_ones(pltpu.roll(kw, shift, 1))
            kh_scr[par][r:r + 8, :] = b
            red = b if (red is None or not _BR) else red | b
        return pltpu.bitcast(red, f32)

    def fix_first(sl, i, start=None):
        out = []
        nc = tiles(nc_scr[sl])
        if start is not None:
            nc = [jnp.where(never(0), start[j], nc[j]) for j in range(NJ)]
        for a in range(2):
            r = 16 * i + 8 * a
            v = tiles(p_scr[sl][r:r + 8, :])
            v = [jnp.exp2(v[j] + nc[j]) for j in range(NJ)]
            p_scr[sl][r:r + 8, :] = jnp.concatenate(v, axis=1)
            out.extend(enumerate(v))
        return out

    def pv_chunk(h, c, sl, acc, tie):
        src = p_scr[sl]
        parts = [src[c * KC + a * 64:c * KC + (a + 1) * 64, :]
                 for a in range(KC // 64)]
        p = jnp.concatenate(parts, axis=0)
        v = vx_scr[h, :, c * KC:(c + 1) * KC]
        for hf in range(2 if tie else 0):
            r0 = (KC - 8, KC // 2 - 8)[hf]
            pt = tiles(p[r0:r0 + 8, :])
            for j in range(NJ):
                ts = [t for jj, t in tie[hf] if jj == j]
                if ts:
                    pt[j] = jnp.where(never(1),
                                      functools.reduce(jnp.maximum, ts), pt[j])
            pieces = [p[0:r0, :], jnp.concatenate(pt, axis=1)] + (
                [p[r0 + 8:, :]] if r0 + 8 < KC else [])
            p = jnp.concatenate(pieces, axis=0)
        o = lax.dot_general(v, p, _NN, preferred_element_type=f32)
        return o if acc is None else o + acc

    def finish(h, qb, o, check):
        off = (DH * h) % 8
        w0 = pl.multiple_of(DH * h - off, 8)
        l = jnp.where(off == 0, o[_VR - 1:_VR, :], o[0:1, :])
        if check:
            bad = jnp.where(jnp.abs(o) < _BIG, 0.0, 1.0)
            bad = jnp.max(bad.reshape(_VR // 8, 8, TQ), axis=0)
            badl = jnp.where((l > _LMIN) & (l < _LMAX), 0.0, 1.0)
            flag_scr[...] = jnp.maximum(flag_scr[...],
                                        jnp.maximum(bad, badl))
        r = pl.reciprocal(l, approx=True)
        r = r * (2.0 - l * r)
        r = r * (2.0 - l * r)
        on = o * r
        valid = (rowv >= off) & (rowv < off + DH)
        pltpu.store(ot_scr.at[qb, pl.ds(w0, _VR), :], on, mask=valid)

    @pl.when(step == 0)
    def _():
        wc = w_copies()
        x_copy(0).start()
        wc[0].start()

        p_scr[1][(NC - _LQ) * KC:, :] = jnp.ones((_LQ * KC, TQ), f32)
        flag_scr[...] = jnp.zeros((8, TQ), f32)
        nc_scr[1] = jnp.zeros((8, TQ), f32)
        kb_scr[1][(NG - 1) * DH:] = jnp.zeros((DH, 8, _LANES), f32)

        def ln1(c, i):
            r = pl.multiple_of(c * TQ + i * _LNR, _LNR)
            xn_scr[pl.ds(r, _LNR), :] = _layernorm_f32(
                x_v[pl.ds(r, _LNR), :].astype(f32)).astype(bf16)

        x_copy(0).wait()
        x_copy(1).start()
        for i in range(TQ // _LNR):
            ln1(0, i)
        wc[0].wait()
        for c in range(2, NQ):
            x_copy(c).start()
        wc[1].start()
        wc[2].start()

        n_early = len([v for v in vchunks if v < (NQ - 1) * (TQ // KC)])

        def kproj(c, carry, last=False):
            if not last:
                x_copy(c + 1).wait()
            else:
                for d in range(DH):
                    build_kb(step, (d, range(n_early)), 0)
            for i in range(TQ // KC):
                r = pl.multiple_of(c * TQ + i * KC, KC)
                k = jnp.dot(xn_scr[pl.ds(r, KC), :], wk_v[...],
                            preferred_element_type=f32).astype(bf16)
                r2 = pl.multiple_of((c * TQ + i * KC) // 2, KC // 2)
                for s in range(NSLAB):
                    a = s * HPS * DH
                    if a + _LANES <= D:
                        blk = k[:, a:a + _LANES]
                    else:
                        blk = jnp.concatenate(
                            [k[:, a:], jnp.zeros((KC, a + _LANES - D), bf16)],
                            axis=1)
                    k_scr[s, pl.ds(r2, KC // 2), :] = pltpu.bitcast(blk, u32)
                    if s == 0:
                        kh_scr[0][pl.ds(r2, KC // 2), :] = with_ones(
                            pltpu.bitcast(blk, u32))
                npc = TQ // _LNR
                for ii in range(npc):
                    if not last and (ii * _LND) // npc == i:
                        ln1(c + 1, ii)
            return carry

        lax.fori_loop(0, NQ - 1, kproj, 0)
        kproj(NQ - 1, 0, True)
        wc[1].wait()
        wc[2].wait()
        for cp in late_copies():
            cp.start()

        row32 = lax.broadcasted_iota(jnp.int32, (32, TQ), 0)

        def qvproj(c, carry):
            r0 = pl.multiple_of(c * TQ, TQ)
            qv = jnp.dot(xn_scr[pl.ds(r0, TQ), :], wqv_v[...],
                         preferred_element_type=f32)
            qvt = qv.T
            vt = qvt[D:, :]
            qs = (qvt[0:D + 32, :] * qscale).astype(bf16).astype(f32)
            for h in range(_H):
                w = qs[h * DH:h * DH + 32, :]
                qm_scr[c, h] = pltpu.bitcast(
                    jnp.where(row32 < DH, w, 0.0).astype(bf16), u32)
                qf_scr[c, h] = w[0:_VR, :]
                w0 = 8 * ((DH * h) // 8)
                ones_row = _VR - 1 if (DH * h) % 8 == 0 else 0
                win = jnp.where(rowv == ones_row, 1.0, vt[w0:w0 + _VR, :])
                vx_scr[h, :, pl.ds(r0, TQ)] = win
            return carry

        lax.fori_loop(0, NQ, qvproj, 0)
        for d in range(DH):
            build_kb(step, (d, range(n_early, n16)), 0)
        estimate(step, 0, 0, 0, 0)
        for i in range(nrows(0) // 16):
            fix_first(0, i)

        NP = _HU * NQ
        vt_all = [(g, j) for g in range(NG) for j in range(NJ)]

        vr = [vrow[2 * i] // 2 for i in range(n16)]
        rest = [r for r in range(0, S // 2, 8) if r not in vr]
        kh_items = [(build_kh, (vr + rest)[a:a + 8])
                    for a in range(0, S // 16, 8)]
        kb_items = [(build_kb, (d, range(a, min(a + 8, n16))))
                    for d in range(DH) for a in range(0, n16, 8)]
        nfirst = -(-n16 // 8) + 1
        items = kh_items[:nfirst]
        kh_rest = kh_items[nfirst:]
        for n, kbi in enumerate(kb_items):
            items.append(kbi)
            while kh_rest and (len(kh_items) - nfirst - len(kh_rest)) * len(
                    kb_items) < (n + 1) * (len(kh_items) - nfirst):
                items.append(kh_rest.pop(0))
        g_last = NG - 1
        js_last = tuple(j for g, j in vt_all[-_NT4:] if g == g_last)

        def body(it, acc_prev):
            h0 = it * _HU
            head = lambda u: jnp.clip(h0 + u // NQ, 0, _H - 1)
            accs = {-1: acc_prev}
            builds = {}
            for i in range(_HU):
                t0 = i * NQ * NC + 1
                t1 = (i + 1) * NQ * NC - 3
                for n, (fn, g) in enumerate(items):
                    t = t0 + (n * (t1 - t0)) // len(items)
                    builds.setdefault(t, []).append(
                        (fn, head((i + 1) * NQ), g, (i + 1) % 2, n))
            due = {}
            start = (None, None)
            for u in range(NP):
                h, qb, par, sl = head(u), u % NQ, (u // NQ) % 2, u % 2
                for s in range(NC):
                    t = u * NC + s
                    if s == _ES:
                        st = estimate(head(u + 1), (u + 1) % NQ,
                                      ((u + 1) // NQ) % 2, 8 + u, 1 - sl)
                    else:
                        st = probs_mxu(h, qb, s + 1 if s < _ES else s, par,
                                       u, sl)
                    mid = [tiles(st[r:r + 8, :]) for r in _TV]
                    for hf in range(2):
                        due.setdefault(t + 1, ([], []))[hf].extend(
                            enumerate(tiles(st[_TE[hf]:_TE[hf] + 8, :])))
                    mine = vt_all[s * _NT4:(s + 1) * _NT4]
                    if t == 0:
                        due.setdefault(1, ([], []))[1].extend(probs_vpu(
                            head(-1), NQ - 1, g_last, js_last, 1, 1, None,
                            NP).items())
                    if _ES + 2 <= s < _ES + 2 + nrows(0) // 16:
                        due.setdefault(t + 1, ([], []))[1].extend(
                            fix_first(1 - sl, s - _ES - 2, start[0]))
                    for n, g in enumerate(sorted(set(g for g, _ in mine))):
                        if t == NP * NC - 1 and g == g_last:
                            continue
                        js = tuple(j for gg, j in mine if gg == g)
                        acc = probs_vpu(h, qb, g, js, par, sl,
                                        start[min(n, 1)], u)
                        due.setdefault(t + _VD, ([], []))[min(n, 1)].extend(
                            acc.items())
                    for (fn, bh, g, bpar, n) in builds.get(t, ()):
                        due.setdefault(t + _BD, ([], []))[n % 2].append(
                            (n % NJ, fn(bh, g, bpar, start[0])))
                    start = mid
                    p = t - _LQ
                    pu, pc = p // NC, p % NC
                    accs[pu] = pv_chunk(head(pu), pc, pu % 2, accs.get(pu),
                                        due.get(t))
                    if pc == NC - 1:
                        finish(head(pu), pu % NQ, accs[pu], True)
            return accs[NP - 1]

        acc3 = lax.fori_loop(0, _H // _HU, body, jnp.zeros((_VR, TQ), f32))
        hl = _H - 1 + step
        probs_vpu(hl, NQ - 1, g_last, js_last, 1, 1, None, NP)
        for pc in range(NC - _LQ, NC):
            acc3 = pv_chunk(hl, pc, 1, acc3, None)
        finish(hl, NQ - 1, acc3, True)

        @pl.when(jnp.max(flag_scr[...]) > 0.0)
        def _():
            def unit(t, carry):
                h = t // NQ
                qb = t % NQ
                shift = (_LANES - (h % HPS) * DH) % _LANES
                w = pltpu.bitcast(qm_scr[qb, h], bf16)

                def pass1(c, m):
                    r2 = pl.multiple_of(c * (KC // 2), KC // 2)
                    kc = pltpu.bitcast(pltpu.roll(
                        k_scr[h // HPS, pl.ds(r2, KC // 2), :], shift, 1),
                        bf16)
                    st = jnp.dot(kc[:, 0:32], w, preferred_element_type=f32)
                    p0_scr[pl.ds(pl.multiple_of(c * KC, KC), KC), :] = st
                    return jnp.maximum(
                        m, jnp.max(st.reshape(KC // 8, 8, TQ), axis=0))

                m = lax.fori_loop(0, NC, pass1,
                                  jnp.full((8, TQ), -jnp.inf, f32))
                m = jnp.max(m, axis=0, keepdims=True)

                def pass2(c, acc):
                    r = pl.multiple_of(c * KC, KC)
                    p = jnp.exp2(p0_scr[pl.ds(r, KC), :] - m)
                    return acc + lax.dot_general(
                        vx_scr[h, :, pl.ds(r, KC)], p, _NN,
                        preferred_element_type=f32)

                finish(h, qb, lax.fori_loop(
                    0, NC, pass2, jnp.zeros((_VR, TQ), f32)), False)
                return carry

            lax.fori_loop(0, _H * NQ, unit, 0)

        for cp in late_copies():
            cp.wait()

    R = TQ // _FS

    def o_copy(st, r):
        return pltpu.make_async_copy(
            o_v.at[st % 2, r],
            o_ref.at[pl.ds(pl.multiple_of(st * TQ + r * R, R), R), :],
            osems.at[(st % 2) * _FS + r])

    @pl.when(step >= 2)
    def _():
        for r in range(_FS):
            o_copy(step - 2, r).wait()

    hres = []
    for r in range(_FS):
        o_nat = ot_scr[step, :, r * R:(r + 1) * R].T.astype(bf16)
        attn = jnp.dot(o_nat, wo_v[...], preferred_element_type=f32)
        q0 = pl.multiple_of(step * TQ + r * R, R)
        hres.append(x_v[pl.ds(q0, R), :].astype(f32) + attn)
    for r in range(_FS):
        hn = _layernorm_f32(hres[r]).astype(bf16)
        gu = lax.dot_general(hn, wgu_v[...], _NT, preferred_element_type=f32)
        g = jnp.concatenate([gu[:, 0:FM], gu[:, 2 * FM:2 * FM + FT]], axis=1)
        u = jnp.concatenate([gu[:, FM:2 * FM], gu[:, 2 * FM + FT:]], axis=1)
        act = (g * jax.nn.sigmoid(g) * u).astype(bf16)
        dn = jnp.dot(act, wd_v[...], preferred_element_type=f32)
        o_v[step % 2, r] = (hres[r] + dn).astype(o_v.dtype)
        o_copy(step, r).start()

    @pl.when(step == NQ - 1)
    def _():
        for r in range(_FS):
            o_copy(step - 1, r).wait()
        for r in range(_FS):
            o_copy(step, r).wait()


@jax.jit
def pallas_sequential_preLN__mha_block__swiglu_ffn__prompt_kernel(
    A_x: jax.Array,
    A_wqkv: jax.Array,
    A_wo: jax.Array,
    B_x: jax.Array,
    B_w_gate: jax.Array,
    B_w_up: jax.Array,
    B_w_down: jax.Array,
):
    del B_x
    B, S, D = A_x.shape
    assert B == 1
    F = B_w_gate.shape[1]
    DH = D // _H
    HPS = _LANES // DH
    NSLAB = -(-_H // HPS)
    NQ = S // _TQ
    x = A_x.reshape(S, D)
    bf16 = jnp.bfloat16
    f32 = jnp.float32
    u32 = jnp.uint32
    nkb = (_NT4 * (S // _KC)) // (_TQ // _LANES) * DH

    kern = functools.partial(_kernel, S=S, D=D, F=F, DH=DH, HPS=HPS,
                             NSLAB=NSLAB)
    out = pl.pallas_call(
        kern,
        grid=(NQ,),
        in_specs=[pl.BlockSpec(memory_space=pl.ANY)] * 6,
        out_specs=pl.BlockSpec(memory_space=pl.ANY),
        out_shape=jax.ShapeDtypeStruct((S, D), A_x.dtype),
        scratch_shapes=[
            pltpu.VMEM((S, D), bf16),
            pltpu.VMEM((D, D), bf16),
            pltpu.VMEM((D, 2 * D), bf16),
            pltpu.VMEM((D, D), bf16),
            pltpu.VMEM((2 * F, D), bf16),
            pltpu.VMEM((F, D), bf16),
            pltpu.VMEM((S, D), bf16),
            pltpu.VMEM((NQ, _H, 16, _TQ), u32),
            pltpu.VMEM((NSLAB, S // 2, _LANES), u32),
            pltpu.VMEM((_H, _VR, S), f32),
            pltpu.VMEM((NQ, D, _TQ), f32),
            pltpu.VMEM((S, _TQ), f32),
            pltpu.VMEM((S, _TQ), f32),
            pltpu.VMEM((NQ, _H, _VR, _TQ), f32),
            pltpu.VMEM((nkb, 8, _LANES), f32),
            pltpu.VMEM((nkb, 8, _LANES), f32),
            pltpu.VMEM((S // 2, _LANES), u32),
            pltpu.VMEM((S // 2, _LANES), u32),
            pltpu.VMEM((2, 8, _TQ), u32),
            pltpu.VMEM((2, 8, _TQ), f32),
            pltpu.VMEM((8, _TQ), f32),
            pltpu.VMEM((2, _FS, _TQ // _FS, D), A_x.dtype),
            pltpu.SemaphoreType.DMA((NQ + 9,)),
            pltpu.SemaphoreType.DMA((2 * _FS,)),
        ],
        compiler_params=pltpu.CompilerParams(
            dimension_semantics=("arbitrary",),
            vmem_limit_bytes=110 * 1024 * 1024,
        ),
    )(x, A_wqkv, A_wo, B_w_gate.T, B_w_up.T, B_w_down)
    return out.reshape(B, S, D)
```

```python
import functools
import math

import jax
import jax.numpy as jnp
from jax import lax
import jax.experimental.pallas as pl
import jax.experimental.pallas.tpu as pltpu

_H = 32
_EPS = 1e-5
_LANES = 128
_TQ = 512
_KC = 128
_VR = 24
_NT4 = 8
_FS = 4
_HU = 2
_LQ = 5
_ES = 6
_TV = (48, 104)
_TE = (16, 72)
_KS = 2
_LND = 1
_LNR = 64
_LMAX = 2.0 ** 40
_LMIN = 2.0 ** -20
_BIG = 3.0e38

_NN = (((1,), (0,)), ((), ()))
_NT = (((1,), (1,)), ((), ()))


def _layernorm_f32(x):
    m = jnp.mean(x, axis=-1, keepdims=True)
    xc = x - m
    v = jnp.mean(xc * xc, axis=-1, keepdims=True)
    return xc * lax.rsqrt(v + _EPS)


def _kernel(x_hbm, wqkv_hbm, wo_hbm, wgt_hbm, wut_hbm, wd_hbm, o_ref,
            x_v, wk_v, wqv_v, wo_v, wgu_v, wd_v,
            xn_scr, qm_scr, k_scr, vx_scr, ot_scr, p0_scr, p1_scr,
            qf_scr, kb0_scr, kb1_scr, kh0_scr, kh1_scr, qc_scr, nc_scr,
            flag_scr, o_v, sems, osems,
            *, S, D, F, DH, HPS, NSLAB):
    step = pl.program_id(0)
    p_scr = (p0_scr, p1_scr)
    kb_scr = (kb0_scr, kb1_scr)
    kh_scr = (kh0_scr, kh1_scr)
    qscale = (DH ** -0.5) * math.log2(math.e)
    TQ, KC = _TQ, _KC
    NC = S // KC
    NQ = S // TQ
    NJ = TQ // _LANES
    FM = (F // _LANES) * _LANES
    FT = F - FM
    bf16 = jnp.bfloat16
    f32 = jnp.float32
    u32 = jnp.uint32
    n16 = (_NT4 * NC) // (2 * NJ)
    vchunks = [c for c in range(NC)
               if ((c + 1) * n16) // NC > (c * n16) // NC]
    assert len(vchunks) == n16
    NG = 2 * n16
    vrow = [vc * KC + KC - 16 + o for vc in vchunks for o in (0, 8)]

    def opaque_zero(h, salt):
        return lax.shift_right_logical(h + salt, 10)

    def x_copy(c):
        return pltpu.make_async_copy(
            x_hbm.at[pl.ds(c * TQ, TQ), :], x_v.at[pl.ds(c * TQ, TQ), :],
            sems.at[c])

    def w_copies():
        return [
            pltpu.make_async_copy(wqkv_hbm.at[:, pl.ds(D, D)], wk_v,
                                  sems.at[NQ]),
            pltpu.make_async_copy(wqkv_hbm.at[:, pl.ds(0, D)],
                                  wqv_v.at[:, pl.ds(0, D)], sems.at[NQ + 1]),
            pltpu.make_async_copy(wqkv_hbm.at[:, pl.ds(2 * D, D)],
                                  wqv_v.at[:, pl.ds(D, D)], sems.at[NQ + 2]),
        ]

    def late_copies():
        b = NQ + 3
        return [
            pltpu.make_async_copy(wo_hbm, wo_v, sems.at[b]),
            pltpu.make_async_copy(wgt_hbm.at[pl.ds(0, FM), :],
                                  wgu_v.at[pl.ds(0, FM), :], sems.at[b + 1]),
            pltpu.make_async_copy(wut_hbm.at[pl.ds(0, FM), :],
                                  wgu_v.at[pl.ds(FM, FM), :], sems.at[b + 2]),
            pltpu.make_async_copy(wgt_hbm.at[pl.ds(FM, FT), :],
                                  wgu_v.at[pl.ds(2 * FM, FT), :],
                                  sems.at[b + 3]),
            pltpu.make_async_copy(wut_hbm.at[pl.ds(FM, FT), :],
                                  wgu_v.at[pl.ds(2 * FM + FT, FT), :],
                                  sems.at[b + 4]),
            pltpu.make_async_copy(wd_hbm, wd_v, sems.at[b + 5]),
        ]

    rowv = lax.broadcasted_iota(jnp.int32, (_VR, TQ), 0)
    row8 = lax.broadcasted_iota(jnp.int32, (8, TQ), 0)
    row8l = lax.broadcasted_iota(jnp.int32, (8, _LANES), 0)

    def never(i):
        return row8l < opaque_zero(step, 200 + i)

    def tiles(v):
        return [v[:, j * _LANES:(j + 1) * _LANES] for j in range(NJ)]

    def with_ones(kw):
        lane = lax.broadcasted_iota(jnp.int32, kw.shape, 1)
        return jnp.where((lane == DH) | (lane == DH + 1),
                         jnp.uint32(0x3F803F80), kw)

    def nrows(c):
        return KC - 16 if c in vchunks else KC

    def qk_dot(h, c, par, salt, w):
        z = pl.multiple_of(opaque_zero(h, 600 + salt) * 8, 8)
        kc = pltpu.bitcast(
            kh_scr[par][pl.ds(z + c * KC // 2, nrows(c) // 2), :], bf16)
        return jnp.dot(kc[:, 0:32], pltpu.bitcast(w, bf16),
                       preferred_element_type=f32)

    def estimate(h, qb, par, salt, sl):
        st = qk_dot(h, 0, par, salt, qm_scr[qb, h])
        p_scr[sl][0:nrows(0), :] = st
        c = jnp.max(jnp.max(st.reshape(nrows(0) // 8, 8, TQ), axis=0),
                    axis=0, keepdims=True)
        hi = c.astype(bf16).astype(f32)
        lo = (c - hi).astype(bf16).astype(f32)
        nc_scr[sl] = jnp.broadcast_to(-(hi + lo), (8, TQ))
        r = DH - 16
        top = jnp.where(row8 < r, qf_scr[qb, h, 16:24, :],
                        jnp.where(row8 == r, -hi,
                                  jnp.where(row8 == r + 1, -lo, 0.0)))
        qc_scr[sl] = pltpu.bitcast(
            jnp.concatenate([top, jnp.zeros((8, TQ), f32)],
                            axis=0).astype(bf16), u32)
        return st

    def probs_mxu(h, qb, c, par, salt, sl):
        w = jnp.concatenate([qm_scr[qb, h, 0:8, :], qc_scr[sl]], axis=0)
        st = qk_dot(h, c, par, salt, w)
        p_scr[sl][c * KC:c * KC + nrows(c), :] = jnp.exp2(st)
        return st

    def probs_vpu(h, qb, g, js, par, sl, start, salt):
        hq = h + opaque_zero(h, 100 + g % 4)
        acc = {}
        for i0 in range(0, len(js), _KS):
            z = opaque_zero(h, 700 + salt * NJ + js[i0])
            for d in range(DH):
                kb = kb_scr[par][z + (g * DH + d)]
                for j in js[i0:i0 + _KS]:
                    t = kb * qf_scr[qb, hq, d:d + 1,
                                    j * _LANES:(j + 1) * _LANES]
                    if j not in acc:
                        acc[j] = nc_scr[sl, :, j * _LANES:(j + 1) * _LANES]
                        if start is not None:
                            acc[j] = jnp.where(never(0), start[j], acc[j])
                    acc[j] = acc[j] + t
        for j in js:
            p_scr[sl][vrow[g]:vrow[g] + 8, j * _LANES:(j + 1) * _LANES] = (
                jnp.exp2(acc[j]))
        return acc

    def build_kb(h, item, par, start=None):
        d, idx = item
        kb_ref = kb_scr[par]
        z = pl.multiple_of(opaque_zero(h, 640 + d) * 8, 8)
        red = None
        for i in idx:
            kw = kh_scr[par][pl.ds(z + vrow[2 * i] // 2, 8), :]
            if start is not None:
                kw = jnp.where(never(0), pltpu.bitcast(start[0], u32), kw)
            b = jnp.broadcast_to(kw[:, d:d + 1], (8, _LANES))
            bf = pltpu.bitcast(b, bf16).astype(f32)
            kb_ref[(2 * i) * DH + d] = bf[0:8]
            kb_ref[(2 * i + 1) * DH + d] = bf[8:16]
            red = b if red is None else red | b
        return pltpu.bitcast(red, f32)

    def build_kh(h, rows, par, start=None):
        shift = (_LANES - (h % HPS) * DH) % _LANES
        red = None
        for r in rows:
            kw = k_scr[h // HPS, r:r + 8, :]
            if start is not None:
                kw = jnp.where(never(0), pltpu.bitcast(start[0], u32), kw)
            b = with_ones(pltpu.roll(kw, shift, 1))
            kh_scr[par][r:r + 8, :] = b
            red = b if red is None else red | b
        return pltpu.bitcast(red, f32)

    def fix_first(sl, i, start=None):
        out = []
        nc = tiles(nc_scr[sl])
        if start is not None:
            nc = [jnp.where(never(0), start[j], nc[j]) for j in range(NJ)]
        for a in range(2):
            r = 16 * i + 8 * a
            v = tiles(p_scr[sl][r:r + 8, :])
            v = [jnp.exp2(v[j] + nc[j]) for j in range(NJ)]
            p_scr[sl][r:r + 8, :] = jnp.concatenate(v, axis=1)
            out.extend(enumerate(v))
        return out

    def pv_chunk(h, c, sl, acc, tie):
        src = p_scr[sl]
        parts = [src[c * KC + a * 64:c * KC + (a + 1) * 64, :]
                 for a in range(KC // 64)]
        p = jnp.concatenate(parts, axis=0)
        v = vx_scr[h, :, c * KC:(c + 1) * KC]
        for hf in range(2 if tie else 0):
            r0 = (KC - 8, KC // 2 - 8)[hf]
            pt = tiles(p[r0:r0 + 8, :])
            for j in range(NJ):
                ts = [t for jj, t in tie[hf] if jj == j]
                if ts:
                    pt[j] = jnp.where(never(1),
                                      functools.reduce(jnp.maximum, ts), pt[j])
            pieces = [p[0:r0, :], jnp.concatenate(pt, axis=1)] + (
                [p[r0 + 8:, :]] if r0 + 8 < KC else [])
            p = jnp.concatenate(pieces, axis=0)
        o = lax.dot_general(v, p, _NN, preferred_element_type=f32)
        return o if acc is None else o + acc

    def finish(h, qb, o, check):
        off = (DH * h) % 8
        w0 = pl.multiple_of(DH * h - off, 8)
        l = jnp.where(off == 0, o[_VR - 1:_VR, :], o[0:1, :])
        if check:
            bad = jnp.where(jnp.abs(o) < _BIG, 0.0, 1.0)
            bad = jnp.max(bad.reshape(_VR // 8, 8, TQ), axis=0)
            badl = jnp.where((l > _LMIN) & (l < _LMAX), 0.0, 1.0)
            flag_scr[...] = jnp.maximum(flag_scr[...],
                                        jnp.maximum(bad, badl))
        r = pl.reciprocal(l, approx=True)
        r = r * (2.0 - l * r)
        r = r * (2.0 - l * r)
        on = o * r
        valid = (rowv >= off) & (rowv < off + DH)
        pltpu.store(ot_scr.at[qb, pl.ds(w0, _VR), :], on, mask=valid)

    @pl.when(step == 0)
    def _():
        wc = w_copies()
        x_copy(0).start()
        wc[0].start()

        p_scr[1][(NC - _LQ) * KC:, :] = jnp.ones((_LQ * KC, TQ), f32)
        flag_scr[...] = jnp.zeros((8, TQ), f32)
        nc_scr[1] = jnp.zeros((8, TQ), f32)
        kb_scr[1][(NG - 1) * DH:] = jnp.zeros((DH, 8, _LANES), f32)

        def ln1(c, i):
            r = pl.multiple_of(c * TQ + i * _LNR, _LNR)
            xn_scr[pl.ds(r, _LNR), :] = _layernorm_f32(
                x_v[pl.ds(r, _LNR), :].astype(f32)).astype(bf16)

        x_copy(0).wait()
        x_copy(1).start()
        for i in range(TQ // _LNR):
            ln1(0, i)
        wc[0].wait()
        for c in range(2, NQ):
            x_copy(c).start()
        wc[1].start()
        wc[2].start()

        n_early = len([v for v in vchunks if v < (NQ - 1) * (TQ // KC)])

        def kproj(c, carry, last=False):
            if not last:
                x_copy(c + 1).wait()
            else:
                for d in range(DH):
                    build_kb(step, (d, range(n_early)), 0)
            for i in range(TQ // KC):
                r = pl.multiple_of(c * TQ + i * KC, KC)
                k = jnp.dot(xn_scr[pl.ds(r, KC), :], wk_v[...],
                            preferred_element_type=f32).astype(bf16)
                r2 = pl.multiple_of((c * TQ + i * KC) // 2, KC // 2)
                for s in range(NSLAB):
                    a = s * HPS * DH
                    if a + _LANES <= D:
                        blk = k[:, a:a + _LANES]
                    else:
                        blk = jnp.concatenate(
                            [k[:, a:], jnp.zeros((KC, a + _LANES - D), bf16)],
                            axis=1)
                    k_scr[s, pl.ds(r2, KC // 2), :] = pltpu.bitcast(blk, u32)
                    if s == 0:
                        kh_scr[0][pl.ds(r2, KC // 2), :] = with_ones(
                            pltpu.bitcast(blk, u32))
                npc = TQ // _LNR
                for ii in range(npc):
                    if not last and (ii * _LND) // npc == i:
                        ln1(c + 1, ii)
            return carry

        lax.fori_loop(0, NQ - 1, kproj, 0)
        kproj(NQ - 1, 0, True)
        wc[1].wait()
        wc[2].wait()
        for cp in late_copies():
            cp.start()

        row32 = lax.broadcasted_iota(jnp.int32, (32, TQ), 0)

        def qvproj(c, carry):
            r0 = pl.multiple_of(c * TQ, TQ)
            qv = jnp.dot(xn_scr[pl.ds(r0, TQ), :], wqv_v[...],
                         preferred_element_type=f32)
            qvt = qv.T
            vt = qvt[D:, :]
            qs = (qvt[0:D + 32, :] * qscale).astype(bf16).astype(f32)
            for h in range(_H):
                w = qs[h * DH:h * DH + 32, :]
                qm_scr[c, h] = pltpu.bitcast(
                    jnp.where(row32 < DH, w, 0.0).astype(bf16), u32)
                qf_scr[c, h] = w[0:_VR, :]
                w0 = 8 * ((DH * h) // 8)
                ones_row = _VR - 1 if (DH * h) % 8 == 0 else 0
                win = jnp.where(rowv == ones_row, 1.0, vt[w0:w0 + _VR, :])
                vx_scr[h, :, pl.ds(r0, TQ)] = win
            return carry

        lax.fori_loop(0, NQ, qvproj, 0)
        for d in range(DH):
            build_kb(step, (d, range(n_early, n16)), 0)
        estimate(step, 0, 0, 0, 0)
        for i in range(nrows(0) // 16):
            fix_first(0, i)

        NP = _HU * NQ
        vt_all = [(g, j) for g in range(NG) for j in range(NJ)]

        vr = [vrow[2 * i] // 2 for i in range(n16)]
        rest = [r for r in range(0, S // 2, 8) if r not in vr]
        kh_items = [(build_kh, (vr + rest)[a:a + 8])
                    for a in range(0, S // 16, 8)]
        kb_items = [(build_kb, (d, range(a, min(a + 8, n16))))
                    for d in range(DH) for a in range(0, n16, 8)]
        nfirst = -(-n16 // 8) + 1
        items = kh_items[:nfirst]
        kh_rest = kh_items[nfirst:]
        for n, kbi in enumerate(kb_items):
            items.append(kbi)
            while kh_rest and (len(kh_items) - nfirst - len(kh_rest)) * len(
                    kb_items) < (n + 1) * (len(kh_items) - nfirst):
                items.append(kh_rest.pop(0))
        g_last = NG - 1
        js_last = tuple(j for g, j in vt_all[-_NT4:] if g == g_last)

        def body(it, acc_prev):
            h0 = it * _HU
            head = lambda u: jnp.clip(h0 + u // NQ, 0, _H - 1)
            accs = {-1: acc_prev}
            builds = {}
            for i in range(_HU):
                t0 = i * NQ * NC + 1
                t1 = (i + 1) * NQ * NC - 3
                for n, (fn, g) in enumerate(items):
                    t = t0 + (n * (t1 - t0)) // len(items)
                    builds.setdefault(t, []).append(
                        (fn, head((i + 1) * NQ), g, (i + 1) % 2, n))
            due = {}
            start = (None, None)
            for u in range(NP):
                h, qb, par, sl = head(u), u % NQ, (u // NQ) % 2, u % 2
                for s in range(NC):
                    t = u * NC + s
                    if s == _ES:
                        st = estimate(head(u + 1), (u + 1) % NQ,
                                      ((u + 1) // NQ) % 2, 8 + u, 1 - sl)
                    else:
                        st = probs_mxu(h, qb, s + 1 if s < _ES else s, par,
                                       u, sl)
                    mid = [tiles(st[r:r + 8, :]) for r in _TV]
                    for hf in range(2):
                        due.setdefault(t + 1, ([], []))[hf].extend(
                            enumerate(tiles(st[_TE[hf]:_TE[hf] + 8, :])))
                    mine = vt_all[s * _NT4:(s + 1) * _NT4]
                    if t == 0:
                        due.setdefault(1, ([], []))[1].extend(probs_vpu(
                            head(-1), NQ - 1, g_last, js_last, 1, 1, None,
                            NP).items())
                    if _ES + 2 <= s < _ES + 2 + nrows(0) // 16:
                        due.setdefault(t + 1, ([], []))[1].extend(
                            fix_first(1 - sl, s - _ES - 2, start[0]))
                    for n, g in enumerate(sorted(set(g for g, _ in mine))):
                        if t == NP * NC - 1 and g == g_last:
                            continue
                        js = tuple(j for gg, j in mine if gg == g)
                        acc = probs_vpu(h, qb, g, js, par, sl,
                                        start[min(n, 1)], u)
                        due.setdefault(t + 1, ([], []))[min(n, 1)].extend(
                            acc.items())
                    for (fn, bh, g, bpar, n) in builds.get(t, ()):
                        due.setdefault(t + 1, ([], []))[n % 2].append(
                            (n % NJ, fn(bh, g, bpar, start[0])))
                    start = mid
                    p = t - _LQ
                    pu, pc = p // NC, p % NC
                    accs[pu] = pv_chunk(head(pu), pc, pu % 2, accs.get(pu),
                                        due.get(t))
                    if pc == NC - 1:
                        finish(head(pu), pu % NQ, accs[pu], True)
            return accs[NP - 1]

        acc3 = lax.fori_loop(0, _H // _HU, body, jnp.zeros((_VR, TQ), f32))
        hl = _H - 1 + step
        probs_vpu(hl, NQ - 1, g_last, js_last, 1, 1, None, NP)
        for pc in range(NC - _LQ, NC):
            acc3 = pv_chunk(hl, pc, 1, acc3, None)
        finish(hl, NQ - 1, acc3, True)

        @pl.when(jnp.max(flag_scr[...]) > 0.0)
        def _():
            def unit(t, carry):
                h = t // NQ
                qb = t % NQ
                shift = (_LANES - (h % HPS) * DH) % _LANES
                w = pltpu.bitcast(qm_scr[qb, h], bf16)

                def pass1(c, m):
                    r2 = pl.multiple_of(c * (KC // 2), KC // 2)
                    kc = pltpu.bitcast(pltpu.roll(
                        k_scr[h // HPS, pl.ds(r2, KC // 2), :], shift, 1),
                        bf16)
                    st = jnp.dot(kc[:, 0:32], w, preferred_element_type=f32)
                    p0_scr[pl.ds(pl.multiple_of(c * KC, KC), KC), :] = st
                    return jnp.maximum(
                        m, jnp.max(st.reshape(KC // 8, 8, TQ), axis=0))

                m = lax.fori_loop(0, NC, pass1,
                                  jnp.full((8, TQ), -jnp.inf, f32))
                m = jnp.max(m, axis=0, keepdims=True)

                def pass2(c, acc):
                    r = pl.multiple_of(c * KC, KC)
                    p = jnp.exp2(p0_scr[pl.ds(r, KC), :] - m)
                    return acc + lax.dot_general(
                        vx_scr[h, :, pl.ds(r, KC)], p, _NN,
                        preferred_element_type=f32)

                finish(h, qb, lax.fori_loop(
                    0, NC, pass2, jnp.zeros((_VR, TQ), f32)), False)
                return carry

            lax.fori_loop(0, _H * NQ, unit, 0)

        for cp in late_copies():
            cp.wait()

    R = TQ // _FS

    def o_copy(st, r):
        return pltpu.make_async_copy(
            o_v.at[st % 2, r],
            o_ref.at[pl.ds(pl.multiple_of(st * TQ + r * R, R), R), :],
            osems.at[(st % 2) * _FS + r])

    @pl.when(step >= 2)
    def _():
        for r in range(_FS):
            o_copy(step - 2, r).wait()

    hres = []
    for r in range(_FS):
        o_nat = ot_scr[step, :, r * R:(r + 1) * R].T.astype(bf16)
        attn = jnp.dot(o_nat, wo_v[...], preferred_element_type=f32)
        q0 = pl.multiple_of(step * TQ + r * R, R)
        hres.append(x_v[pl.ds(q0, R), :].astype(f32) + attn)
    for r in range(_FS):
        hn = _layernorm_f32(hres[r]).astype(bf16)
        gu = lax.dot_general(hn, wgu_v[...], _NT, preferred_element_type=f32)
        g = jnp.concatenate([gu[:, 0:FM], gu[:, 2 * FM:2 * FM + FT]], axis=1)
        u = jnp.concatenate([gu[:, FM:2 * FM], gu[:, 2 * FM + FT:]], axis=1)
        act = (g * jax.nn.sigmoid(g) * u).astype(bf16)
        dn = jnp.dot(act, wd_v[...], preferred_element_type=f32)
        o_v[step % 2, r] = (hres[r] + dn).astype(o_v.dtype)
        o_copy(step, r).start()

    @pl.when(step == NQ - 1)
    def _():
        for r in range(_FS):
            o_copy(step - 1, r).wait()
        for r in range(_FS):
            o_copy(step, r).wait()


@jax.jit
def pallas_sequential_preLN__mha_block__swiglu_ffn__prompt_kernel(
    A_x: jax.Array,
    A_wqkv: jax.Array,
    A_wo: jax.Array,
    B_x: jax.Array,
    B_w_gate: jax.Array,
    B_w_up: jax.Array,
    B_w_down: jax.Array,
):
    del B_x
    B, S, D = A_x.shape
    assert B == 1
    F = B_w_gate.shape[1]
    DH = D // _H
    HPS = _LANES // DH
    NSLAB = -(-_H // HPS)
    NQ = S // _TQ
    x = A_x.reshape(S, D)
    bf16 = jnp.bfloat16
    f32 = jnp.float32
    u32 = jnp.uint32
    nkb = (_NT4 * (S // _KC)) // (_TQ // _LANES) * DH

    kern = functools.partial(_kernel, S=S, D=D, F=F, DH=DH, HPS=HPS,
                             NSLAB=NSLAB)
    out = pl.pallas_call(
        kern,
        grid=(NQ,),
        in_specs=[pl.BlockSpec(memory_space=pl.ANY)] * 6,
        out_specs=pl.BlockSpec(memory_space=pl.ANY),
        out_shape=jax.ShapeDtypeStruct((S, D), A_x.dtype),
        scratch_shapes=[
            pltpu.VMEM((S, D), bf16),
            pltpu.VMEM((D, D), bf16),
            pltpu.VMEM((D, 2 * D), bf16),
            pltpu.VMEM((D, D), bf16),
            pltpu.VMEM((2 * F, D), bf16),
            pltpu.VMEM((F, D), bf16),
            pltpu.VMEM((S, D), bf16),
            pltpu.VMEM((NQ, _H, 16, _TQ), u32),
            pltpu.VMEM((NSLAB, S // 2, _LANES), u32),
            pltpu.VMEM((_H, _VR, S), f32),
            pltpu.VMEM((NQ, D, _TQ), f32),
            pltpu.VMEM((S, _TQ), f32),
            pltpu.VMEM((S, _TQ), f32),
            pltpu.VMEM((NQ, _H, _VR, _TQ), f32),
            pltpu.VMEM((nkb, 8, _LANES), f32),
            pltpu.VMEM((nkb, 8, _LANES), f32),
            pltpu.VMEM((S // 2, _LANES), u32),
            pltpu.VMEM((S // 2, _LANES), u32),
            pltpu.VMEM((2, 8, _TQ), u32),
            pltpu.VMEM((2, 8, _TQ), f32),
            pltpu.VMEM((8, _TQ), f32),
            pltpu.VMEM((2, _FS, _TQ // _FS, D), A_x.dtype),
            pltpu.SemaphoreType.DMA((NQ + 9,)),
            pltpu.SemaphoreType.DMA((2 * _FS,)),
        ],
        compiler_params=pltpu.CompilerParams(
            dimension_semantics=("arbitrary",),
            vmem_limit_bytes=110 * 1024 * 1024,
        ),
    )(x, A_wqkv, A_wo, B_w_gate.T, B_w_up.T, B_w_down)
    return out.reshape(B, S, D)
```

```python
import functools
import math

import jax
import jax.numpy as jnp
from jax import lax
import jax.experimental.pallas as pl
import jax.experimental.pallas.tpu as pltpu

_H = 32
_EPS = 1e-5
_LANES = 128
_TQ = 512
_KC = 128
_VR = 24
_FS = 4
_HU = 2
_LQ = 7
_ES = 7
_TV = (48, 104)
_TE = (16, 80)
_PK = 1
_PQ = 1
_QS = 2
_QN = 4
_DG = 5
_KS = 2
_LND = 1
_LNR = 64
_LMAX = 2.0 ** 40
_LMIN = 2.0 ** -20
_BIG = 3.0e38

_NN = (((1,), (0,)), ((), ()))
_NT = (((1,), (1,)), ((), ()))


def _layernorm_f32(x):
    m = jnp.mean(x, axis=-1, keepdims=True)
    xc = x - m
    v = jnp.mean(xc * xc, axis=-1, keepdims=True)
    return xc * lax.rsqrt(v + _EPS)


def _kernel(x_hbm, wqkv_hbm, wo_hbm, wgt_hbm, wut_hbm, wd_hbm, o_ref,
            x_v, wk_v, wqv_v, wo_v, wgu_v, wd_v,
            xn_scr, qm_scr, k_scr, vx_scr, ot_scr, p0_scr, p1_scr,
            qf_scr, kb0_scr, kb1_scr, kh0_scr, kh1_scr, qc_scr, nc_scr,
            flag_scr, qb0_scr, qb1_scr, kv0_scr, kv1_scr, o_v, sems, osems,
            *, S, D, F, DH, HPS, NSLAB):
    step = pl.program_id(0)
    p_scr = (p0_scr, p1_scr)
    kb_scr = (kb0_scr, kb1_scr)
    qb_scr = (qb0_scr, qb1_scr)
    kv_scr = (kv0_scr, kv1_scr)
    kh_scr = (kh0_scr, kh1_scr)
    qscale = (DH ** -0.5) * math.log2(math.e)
    TQ, KC = _TQ, _KC
    NC = S // KC
    NQ = S // TQ
    NJ = TQ // _LANES
    FM = (F // _LANES) * _LANES
    FT = F - FM
    bf16 = jnp.bfloat16
    f32 = jnp.float32
    u32 = jnp.uint32
    NG = 2 * NC

    def opaque_zero(h, salt):
        return lax.shift_right_logical(h + salt, 10)

    def x_copy(c):
        return pltpu.make_async_copy(
            x_hbm.at[pl.ds(c * TQ, TQ), :], x_v.at[pl.ds(c * TQ, TQ), :],
            sems.at[c])

    def w_copies():
        return [
            pltpu.make_async_copy(wqkv_hbm.at[:, pl.ds(D, D)], wk_v,
                                  sems.at[NQ]),
            pltpu.make_async_copy(wqkv_hbm.at[:, pl.ds(0, D)],
                                  wqv_v.at[:, pl.ds(0, D)], sems.at[NQ + 1]),
            pltpu.make_async_copy(wqkv_hbm.at[:, pl.ds(2 * D, D)],
                                  wqv_v.at[:, pl.ds(D, D)], sems.at[NQ + 2]),
        ]

    def late_copies():
        b = NQ + 3
        return [
            pltpu.make_async_copy(wo_hbm, wo_v, sems.at[b]),
            pltpu.make_async_copy(wgt_hbm.at[pl.ds(0, FM), :],
                                  wgu_v.at[pl.ds(0, FM), :], sems.at[b + 1]),
            pltpu.make_async_copy(wut_hbm.at[pl.ds(0, FM), :],
                                  wgu_v.at[pl.ds(FM, FM), :], sems.at[b + 2]),
            pltpu.make_async_copy(wgt_hbm.at[pl.ds(FM, FT), :],
                                  wgu_v.at[pl.ds(2 * FM, FT), :],
                                  sems.at[b + 3]),
            pltpu.make_async_copy(wut_hbm.at[pl.ds(FM, FT), :],
                                  wgu_v.at[pl.ds(2 * FM + FT, FT), :],
                                  sems.at[b + 4]),
            pltpu.make_async_copy(wd_hbm, wd_v, sems.at[b + 5]),
        ]

    rowv = lax.broadcasted_iota(jnp.int32, (_VR, TQ), 0)
    row8 = lax.broadcasted_iota(jnp.int32, (8, TQ), 0)

    cache = {}

    def new_scope():
        cache.clear()

    def tile_mask(key, shape, make):
        if key not in cache:
            cache[key] = make()
        if (key, shape) not in cache:
            m = cache[key]
            if shape[1] > _LANES:
                m = jnp.concatenate([m] * (shape[1] // _LANES), axis=1)
            if shape[0] > 8:
                m = jnp.concatenate([m] * (shape[0] // 8), axis=0)
            cache[key, shape] = m
        return cache[key, shape]

    def never(shape, i=0):
        return tile_mask(("never", i), shape, lambda: (
            lax.broadcasted_iota(jnp.int32, (8, _LANES), 0)
            < opaque_zero(step, 200 + i)))

    def ones_lanes(shape):
        def make():
            lane = lax.broadcasted_iota(jnp.int32, (8, _LANES), 1)
            return (lane == DH) | (lane == DH + 1)
        return tile_mask("ones", shape, make)

    def with_ones(kw):
        return lax.select(ones_lanes(kw.shape),
                          jnp.full(kw.shape, 0x3F803F80, u32), kw)

    def gate(start, v):
        if start is None:
            return v
        t = start[:, 0:v.shape[-1]]
        if v.dtype != t.dtype:
            t = pltpu.bitcast(t, v.dtype)
        if v.shape[0] != 8:
            t = jnp.broadcast_to(t[None], (v.shape[0] // 8,) + t.shape
                                 ).reshape(v.shape)
        return lax.select(never(v.shape), t, v)

    def fold(w):
        g = [w[a:a + 8, :] for a in range(0, w.shape[0], 8)]
        return pltpu.bitcast(functools.reduce(jnp.bitwise_or, g), f32)

    NR = KC - 16

    def qk_dot(z, c, par, w):
        kc = pltpu.bitcast(
            kh_scr[par][pl.ds(z + c * KC // 2, NR // 2), :], bf16)
        return jnp.dot(kc[:, 0:32], pltpu.bitcast(w, bf16),
                       preferred_element_type=f32)

    def row_zero(h, salt):
        return pl.multiple_of(opaque_zero(h, salt) * 8, 8)

    def estimate(h, qb, par, salt, sl):
        st = qk_dot(row_zero(h, 600 + salt), 0, par, qm_scr[qb, h])
        p_scr[sl][0:NR, :] = st
        c = jnp.max(jnp.max(st.reshape(NR // 8, 8, TQ), axis=0),
                    axis=0, keepdims=True)
        hi = c.astype(bf16).astype(f32)
        lo = (c - hi).astype(bf16).astype(f32)
        nc_scr[sl] = jnp.broadcast_to(-(hi + lo), (8, TQ))
        r = DH - 16
        top = jnp.where(row8 < r, qf_scr[qb, h, 16:24, :],
                        jnp.where(row8 == r, -hi,
                                  jnp.where(row8 == r + 1, -lo, 0.0)))
        qc_scr[sl] = pltpu.bitcast(
            jnp.concatenate([top, jnp.zeros((8, TQ), f32)],
                            axis=0).astype(bf16), u32)
        return st

    def probs_mxu(h, qb, c, par, z, sl):
        w = jnp.concatenate([qm_scr[qb, h, 0:8, :], qc_scr[sl]], axis=0)
        st = qk_dot(z, c, par, w)
        p_scr[sl][c * KC:c * KC + NR, :] = jnp.exp2(st)
        return st

    def probs_vpu(zs, g, par, sl, start):
        a0 = gate(start, nc_scr[sl])
        out = []
        for n, j0 in enumerate(range(0, NJ, _KS)):
            a = jnp.stack([a0[:, j * _LANES:(j + 1) * _LANES]
                           for j in range(j0, j0 + _KS)])[:, None]
            gk = pl.ds(zs[n] + g, 1)
            jq = pl.ds(zs[2 + g % 4][n], _KS)
            for d0 in range(0, DH, _DG):
                t = (kb_scr[par][gk, d0:d0 + _DG]
                     * qb_scr[sl][jq, d0:d0 + _DG])
                a = jnp.sum(jnp.concatenate([a, t], axis=1), axis=1,
                            keepdims=True)
            out.extend(a[i, 0] for i in range(_KS))
        a = jnp.concatenate(out, axis=1)
        r = (g // 2) * KC + NR + (g % 2) * 8
        p_scr[sl][r:r + 8, :] = jnp.exp2(a)
        return a

    def spread_q(h, qb, sl, ds):
        red = None
        for d in ds:
            v = jnp.stack(
                [jnp.broadcast_to(
                    qf_scr[qb, h, d:d + 1, j * _LANES:(j + 1) * _LANES],
                    (8, _LANES)) for j in range(NJ)])
            qb_scr[sl][:, d] = v
            red = v if red is None else jnp.maximum(red, v)
        return jnp.concatenate([red[j] for j in range(NJ)], axis=1)

    def build_kv(h, item, par, start=None):
        shift = (_LANES - (h % HPS) * DH) % _LANES
        kw = jnp.concatenate(
            [k_scr[h // HPS, (c * KC + NR) // 2:(c + 1) * KC // 2, :]
             for c in range(item, item + 8)], axis=0)
        b = pltpu.roll(gate(start, kw), shift, 1)
        kv_scr[par][item * 8:item * 8 + 64, :] = b
        return fold(b)

    def build_kb(h, item, par, start=None):
        d, c0, n = item
        kw = kv_scr[par][pl.ds(row_zero(h, 640 + d) + c0 * 8, n * 8), :]
        b = jnp.broadcast_to(gate(start, kw)[:, d:d + 1], (n * 8, _LANES))
        kb_scr[par][2 * c0:2 * (c0 + n), d] = pltpu.bitcast(
            b, bf16).astype(f32).reshape(2 * n, 8, _LANES)
        return fold(b)

    def build_kh(h, c, par, start=None):
        shift = (_LANES - (h % HPS) * DH) % _LANES
        r = c * KC // 2
        kw = gate(start, k_scr[h // HPS, r:r + NR // 2, :])
        b = with_ones(pltpu.roll(kw, shift, 1))
        kh_scr[par][r:r + NR // 2, :] = b
        return fold(b)

    def fix_first(sl, i, start=None):
        v = (p_scr[sl][16 * i:16 * i + 16, :].reshape(2, 8, TQ)
             + gate(start, nc_scr[sl])[None])
        v = jnp.exp2(v)
        p_scr[sl][16 * i:16 * i + 16, :] = v.reshape(16, TQ)
        return jnp.max(v, axis=0)

    def pv_chunk(h, c, sl, acc, tie):
        parts = []
        for hf in (1, 0):
            r = c * KC + (1 - hf) * (KC // 2)
            ph = p_scr[sl][r:r + KC // 2, :]
            if not tie:
                parts.append(ph)
                continue
            wide = [t for t in tie[hf] if t.shape[1] == TQ]
            tv = functools.reduce(jnp.maximum, wide)
            for t in tie[hf]:
                if t.shape[1] != TQ:
                    tv = jnp.concatenate(
                        [jnp.maximum(tv[:, 0:_LANES], t), tv[:, _LANES:]],
                        axis=1)
            parts.append(ph[0:KC // 2 - 8, :])
            parts.append(lax.select(never((8, TQ), 1), tv,
                                    ph[KC // 2 - 8:, :]))
        o = lax.dot_general(vx_scr[h, :, c * KC:(c + 1) * KC],
                            jnp.concatenate(parts, axis=0), _NN,
                            preferred_element_type=f32)
        return o if acc is None else o + acc

    def finish(h, qb, o, check):
        off = (DH * h) % 8
        w0 = pl.multiple_of(DH * h - off, 8)
        l = jnp.where(off == 0, o[_VR - 1:_VR, :], o[0:1, :])
        if check:
            bad = jnp.where(jnp.abs(o) < _BIG, 0.0, 1.0)
            bad = jnp.max(bad.reshape(_VR // 8, 8, TQ), axis=0)
            badl = jnp.where((l > _LMIN) & (l < _LMAX), 0.0, 1.0)
            flag_scr[...] = jnp.maximum(flag_scr[...],
                                        jnp.maximum(bad, badl))
        r = pl.reciprocal(l, approx=True)
        r = r * (2.0 - l * r)
        r = r * (2.0 - l * r)
        on = o * r
        valid = (rowv >= off) & (rowv < off + DH)
        pltpu.store(ot_scr.at[qb, pl.ds(w0, _VR), :], on, mask=valid)

    @pl.when(step == 0)
    def _():
        wc = w_copies()
        x_copy(0).start()
        wc[0].start()

        p_scr[1][(NC - _LQ) * KC:, :] = jnp.ones((_LQ * KC, TQ), f32)
        flag_scr[...] = jnp.zeros((8, TQ), f32)
        nc_scr[1] = jnp.zeros((8, TQ), f32)
        qb_scr[1][:, 0:DH] = jnp.zeros((NJ, DH, 8, _LANES), f32)
        kb_scr[1][NG - 1, 0:DH] = jnp.zeros((DH, 8, _LANES), f32)

        def ln1(c, i):
            r = pl.multiple_of(c * TQ + i * _LNR, _LNR)
            xn_scr[pl.ds(r, _LNR), :] = _layernorm_f32(
                x_v[pl.ds(r, _LNR), :].astype(f32)).astype(bf16)

        x_copy(0).wait()
        x_copy(1).start()
        for i in range(TQ // _LNR):
            ln1(0, i)
        wc[0].wait()
        for c in range(2, NQ):
            x_copy(c).start()
        wc[1].start()
        wc[2].start()

        n_early = (NQ - 1) * (TQ // KC)

        def kproj(c, carry, last=False):
            new_scope()
            if not last:
                x_copy(c + 1).wait()
            else:
                for d in range(DH):
                    build_kb(step, (d, 0, n_early), 0)
            for i in range(TQ // KC):
                r = pl.multiple_of(c * TQ + i * KC, KC)
                k = jnp.dot(xn_scr[pl.ds(r, KC), :], wk_v[...],
                            preferred_element_type=f32).astype(bf16)
                r2 = pl.multiple_of((c * TQ + i * KC) // 2, KC // 2)
                for s in range(NSLAB):
                    a = s * HPS * DH
                    if a + _LANES <= D:
                        blk = k[:, a:a + _LANES]
                    else:
                        blk = jnp.concatenate(
                            [k[:, a:], jnp.zeros((KC, a + _LANES - D), bf16)],
                            axis=1)
                    k_scr[s, pl.ds(r2, KC // 2), :] = pltpu.bitcast(blk, u32)
                    if s == 0:
                        kw = pltpu.bitcast(blk, u32)
                        kh_scr[0][pl.ds(r2, NR // 2), :] = with_ones(
                            kw[0:NR // 2, :])
                        rv = pl.multiple_of((c * (TQ // KC) + i) * 8, 8)
                        kv_scr[0][pl.ds(rv, 8), :] = kw[NR // 2:, :]
                npc = TQ // _LNR
                for ii in range(npc):
                    if not last and (ii * _LND) // npc == i:
                        ln1(c + 1, ii)
            return carry

        lax.fori_loop(0, NQ - 1, kproj, 0)
        kproj(NQ - 1, 0, True)
        wc[1].wait()
        wc[2].wait()
        for cp in late_copies():
            cp.start()

        row32 = lax.broadcasted_iota(jnp.int32, (32, TQ), 0)

        def qvproj(c, carry):
            r0 = pl.multiple_of(c * TQ, TQ)
            qv = jnp.dot(xn_scr[pl.ds(r0, TQ), :], wqv_v[...],
                         preferred_element_type=f32)
            qvt = qv.T
            vt = qvt[D:, :]
            qs = (qvt[0:D + 32, :] * qscale).astype(bf16).astype(f32)
            for h in range(_H):
                w = qs[h * DH:h * DH + 32, :]
                qm_scr[c, h] = pltpu.bitcast(
                    jnp.where(row32 < DH, w, 0.0).astype(bf16), u32)
                qf_scr[c, h] = w[0:_VR, :]
                w0 = 8 * ((DH * h) // 8)
                ones_row = _VR - 1 if (DH * h) % 8 == 0 else 0
                win = jnp.where(rowv == ones_row, 1.0, vt[w0:w0 + _VR, :])
                vx_scr[h, :, pl.ds(r0, TQ)] = win
            return carry

        lax.fori_loop(0, NQ, qvproj, 0)
        for d in range(DH):
            build_kb(step, (d, n_early, NC - n_early), 0)
        estimate(step, 0, 0, 0, 0)
        spread_q(step, 0, 0, range(DH))
        for i in range(NR // 16):
            fix_first(0, i)

        NP = _HU * NQ

        kh_items = [(build_kh, c) for c in range(NC)]
        kb_items = [(build_kb, (d, c0, 8))
                    for d in range(DH) for c0 in range(0, NC, 8)]
        items = [(build_kv, c0) for c0 in range(0, NC, 8)] + kh_items[:1]
        done = 1
        for n, kbi in enumerate(kb_items):
            items.append(kbi)
            while (done - 1) * len(kb_items) < (n + 1) * (NC - 1):
                items.append(kh_items[done])
                done += 1

        def zeros6(h, salt):
            z = [opaque_zero(h, 700 + salt * 8 + n) for n in range(6)]
            return z[:2] + [[v + j0 for j0 in range(0, NJ, _KS)]
                            for v in z[2:]]

        def body(it, acc_prev):
            new_scope()
            h0 = it * _HU
            heads = {i: jnp.clip(h0 + i, 0, _H - 1)
                     for i in range(-1, _HU + 1)}
            head = lambda u: heads[u // NQ]
            accs = {-1: acc_prev}
            builds = {}
            for i in range(_HU):
                t0 = i * NQ * NC + 1
                t1 = (i + 1) * NQ * NC - 3
                for n, (fn, g) in enumerate(items):
                    t = t0 + (n * (t1 - t0)) // len(items)
                    builds.setdefault(t, []).append(
                        (fn, heads[i + 1], g, (i + 1) % 2, n))
            due = {}
            start = (None, None)
            for u in range(NP):
                h, qb, par, sl = head(u), u % NQ, (u // NQ) % 2, u % 2
                zk = row_zero(h, 600 + u)
                zs = zeros6(h, u)
                for s in range(NC):
                    t = u * NC + s
                    nxt = due.setdefault(t + 1, ([], []))
                    if s == _ES:
                        st = estimate(head(u + 1), (u + 1) % NQ,
                                      ((u + 1) // NQ) % 2, 8 + u, 1 - sl)
                    else:
                        st = probs_mxu(h, qb, s + 1 if s < _ES else s, par,
                                       zk, sl)
                    for hf in range(2):
                        nxt[hf].append(st[_TE[hf]:_TE[hf] + 8, :])
                    if t == 0:
                        nxt[1].append(probs_vpu(zeros6(h, NP), NG - 1, 1, 1,
                                                None))
                    if _QS <= s < _QS + DH // _QN:
                        nxt[0].append(spread_q(
                            head(u + 1), (u + 1) % NQ, 1 - sl,
                            range((s - _QS) * _QN, (s - _QS + 1) * _QN)))
                    if _ES + 2 <= s < _ES + 2 + NR // 16:
                        nxt[1].append(
                            fix_first(1 - sl, s - _ES - 2, start[0]))
                    for hf in range(2):
                        if t < NP * NC - 1 or hf == 0:
                            nxt[hf].append(probs_vpu(zs, 2 * s + hf, par, sl,
                                                     start[hf]))
                    for (fn, bh, g, bpar, n) in builds.get(t, ()):
                        nxt[n % 2].append(fn(bh, g, bpar, start[0]))
                    start = [st[r:r + 8, :] for r in _TV]
                    p = t - _LQ
                    pu, pc = p // NC, p % NC
                    accs[pu] = pv_chunk(head(pu), pc, pu % 2, accs.get(pu),
                                        due.get(t))
                    if pc == NC - 1:
                        finish(head(pu), pu % NQ, accs[pu], True)
            return accs[NP - 1]

        acc3 = lax.fori_loop(0, _H // _HU, body, jnp.zeros((_VR, TQ), f32))
        new_scope()
        hl = _H - 1 + step
        probs_vpu(zeros6(hl, NP), NG - 1, 1, 1, None)
        for pc in range(NC - _LQ, NC):
            acc3 = pv_chunk(hl, pc, 1, acc3, None)
        finish(hl, NQ - 1, acc3, True)

        @pl.when(jnp.max(flag_scr[...]) > 0.0)
        def _():
            def unit(t, carry):
                h = t // NQ
                qb = t % NQ
                shift = (_LANES - (h % HPS) * DH) % _LANES
                w = pltpu.bitcast(qm_scr[qb, h], bf16)

                def pass1(c, m):
                    r2 = pl.multiple_of(c * (KC // 2), KC // 2)
                    kc = pltpu.bitcast(pltpu.roll(
                        k_scr[h // HPS, pl.ds(r2, KC // 2), :], shift, 1),
                        bf16)
                    st = jnp.dot(kc[:, 0:32], w, preferred_element_type=f32)
                    p0_scr[pl.ds(pl.multiple_of(c * KC, KC), KC), :] = st
                    return jnp.maximum(
                        m, jnp.max(st.reshape(KC // 8, 8, TQ), axis=0))

                m = lax.fori_loop(0, NC, pass1,
                                  jnp.full((8, TQ), -jnp.inf, f32))
                m = jnp.max(m, axis=0, keepdims=True)

                def pass2(c, acc):
                    r = pl.multiple_of(c * KC, KC)
                    p = jnp.exp2(p0_scr[pl.ds(r, KC), :] - m)
                    return acc + lax.dot_general(
                        vx_scr[h, :, pl.ds(r, KC)], p, _NN,
                        preferred_element_type=f32)

                finish(h, qb, lax.fori_loop(
                    0, NC, pass2, jnp.zeros((_VR, TQ), f32)), False)
                return carry

            lax.fori_loop(0, _H * NQ, unit, 0)

        for cp in late_copies():
            cp.wait()

    R = TQ // _FS

    def o_copy(st, r):
        return pltpu.make_async_copy(
            o_v.at[st % 2, r],
            o_ref.at[pl.ds(pl.multiple_of(st * TQ + r * R, R), R), :],
            osems.at[(st % 2) * _FS + r])

    @pl.when(step >= 2)
    def _():
        for r in range(_FS):
            o_copy(step - 2, r).wait()

    hres = []
    for r in range(_FS):
        o_nat = ot_scr[step, :, r * R:(r + 1) * R].T.astype(bf16)
        attn = jnp.dot(o_nat, wo_v[...], preferred_element_type=f32)
        q0 = pl.multiple_of(step * TQ + r * R, R)
        hres.append(x_v[pl.ds(q0, R), :].astype(f32) + attn)
    for r in range(_FS):
        hn = _layernorm_f32(hres[r]).astype(bf16)
        gu = lax.dot_general(hn, wgu_v[...], _NT, preferred_element_type=f32)
        g = jnp.concatenate([gu[:, 0:FM], gu[:, 2 * FM:2 * FM + FT]], axis=1)
        u = jnp.concatenate([gu[:, FM:2 * FM], gu[:, 2 * FM + FT:]], axis=1)
        act = (g * jax.nn.sigmoid(g) * u).astype(bf16)
        dn = jnp.dot(act, wd_v[...], preferred_element_type=f32)
        o_v[step % 2, r] = (hres[r] + dn).astype(o_v.dtype)
        o_copy(step, r).start()

    @pl.when(step == NQ - 1)
    def _():
        for r in range(_FS):
            o_copy(step - 1, r).wait()
        for r in range(_FS):
            o_copy(step, r).wait()


@jax.jit
def pallas_sequential_preLN__mha_block__swiglu_ffn__prompt_kernel(
    A_x: jax.Array,
    A_wqkv: jax.Array,
    A_wo: jax.Array,
    B_x: jax.Array,
    B_w_gate: jax.Array,
    B_w_up: jax.Array,
    B_w_down: jax.Array,
):
    del B_x
    B, S, D = A_x.shape
    assert B == 1
    F = B_w_gate.shape[1]
    DH = D // _H
    HPS = _LANES // DH
    NSLAB = -(-_H // HPS)
    NQ = S // _TQ
    x = A_x.reshape(S, D)
    bf16 = jnp.bfloat16
    f32 = jnp.float32
    u32 = jnp.uint32
    NC = S // _KC

    kern = functools.partial(_kernel, S=S, D=D, F=F, DH=DH, HPS=HPS,
                             NSLAB=NSLAB)
    out = pl.pallas_call(
        kern,
        grid=(NQ,),
        in_specs=[pl.BlockSpec(memory_space=pl.ANY)] * 6,
        out_specs=pl.BlockSpec(memory_space=pl.ANY),
        out_shape=jax.ShapeDtypeStruct((S, D), A_x.dtype),
        scratch_shapes=[
            pltpu.VMEM((S, D), bf16),
            pltpu.VMEM((D, D), bf16),
            pltpu.VMEM((D, 2 * D), bf16),
            pltpu.VMEM((D, D), bf16),
            pltpu.VMEM((2 * F, D), bf16),
            pltpu.VMEM((F, D), bf16),
            pltpu.VMEM((S, D), bf16),
            pltpu.VMEM((NQ, _H, 16, _TQ), u32),
            pltpu.VMEM((NSLAB, S // 2, _LANES), u32),
            pltpu.VMEM((_H, _VR, S), f32),
            pltpu.VMEM((NQ, D, _TQ), f32),
            pltpu.VMEM((S, _TQ), f32),
            pltpu.VMEM((S, _TQ), f32),
            pltpu.VMEM((NQ, _H, _VR, _TQ), f32),
            pltpu.VMEM((2 * NC, DH + _PK, 8, _LANES), f32),
            pltpu.VMEM((2 * NC, DH + _PK, 8, _LANES), f32),
            pltpu.VMEM((S // 2, _LANES), u32),
            pltpu.VMEM((S // 2, _LANES), u32),
            pltpu.VMEM((2, 8, _TQ), u32),
            pltpu.VMEM((2, 8, _TQ), f32),
            pltpu.VMEM((8, _TQ), f32),
            pltpu.VMEM((_TQ // _LANES, DH + _PQ, 8, _LANES), f32),
            pltpu.VMEM((_TQ // _LANES, DH + _PQ, 8, _LANES), f32),
            pltpu.VMEM((8 * NC, _LANES), u32),
            pltpu.VMEM((8 * NC, _LANES), u32),
            pltpu.VMEM((2, _FS, _TQ // _FS, D), A_x.dtype),
            pltpu.SemaphoreType.DMA((NQ + 9,)),
            pltpu.SemaphoreType.DMA((2 * _FS,)),
        ],
        compiler_params=pltpu.CompilerParams(
            dimension_semantics=("arbitrary",),
            vmem_limit_bytes=110 * 1024 * 1024,
        ),
    )(x, A_wqkv, A_wo, B_w_gate.T, B_w_up.T, B_w_down)
    return out.reshape(B, S, D)
```
